```python
import os as _os
_os.environ.setdefault("JAX_PLATFORMS", "cpu")
import jax
import jax.numpy as jnp

def _softmax(x, axis=-1):
    return jax.nn.softmax(x, axis=axis)
def _gelu(x):
    return jax.nn.gelu(x, approximate=True)
def _silu(x):
    return jax.nn.silu(x)
def _sigmoid(x):
    return jax.nn.sigmoid(x)
def _layernorm(x, axis=-1, eps=1e-5):
    m = jnp.mean(x, axis=axis, keepdims=True)
    v = jnp.var(x, axis=axis, keepdims=True)
    return (x - m) / jnp.sqrt(v + eps)
def _scatter_add(tgt, idx, src, axis=0):
    return tgt.at[idx].add(src)
def _segment_sum(src, seg, n):
    return jax.ops.segment_sum(src, seg, n)
class _Rng:
    def __init__(self, key):
        self._k = key
    def _next(self):
        self._k, sub = jax.random.split(self._k)
        return sub
    def normal(self, shape):
        return jax.random.normal(self._next(), shape, dtype=jnp.bfloat16)
    def randint(self, lo, hi, shape):
        return jax.random.randint(self._next(), shape, lo, hi, dtype=jnp.int32)
    def uniform(self, shape, lo=0.0, hi=1.0):
        return jax.random.uniform(self._next(), shape, jnp.bfloat16, lo, hi)
    def permutation(self, n):
        return jax.random.permutation(self._next(), n)


kernel_name = 'gated_mix__softmax_full_mha__dense_activation_relu__prompt'

def setup_inputs():
    _rng = _Rng(jax.random.key(int.from_bytes(__import__("os").urandom(4), "little")))
    _w = (lambda a: (lambda t: t.astype(jnp.bfloat16) if jnp.issubdtype(t.dtype, jnp.floating) else t)(jnp.asarray(a)))
    def _A_setup():
        B, S, D = 1, 2048, 640
        return {
            "x": _w((lambda *s: _rng.normal(s) * 0.05)(B, S, D)),
            "wqkv": _w((lambda *s: _rng.normal(s) * 0.8)(D, 3 * D)),
            "wo": _w((lambda *s: _rng.normal(s) * 0.05)(D, D)),
        }
    _A_in = _A_setup()

    def _B_setup():
        B, S, D, Dff = 1, 2048, 640, 1536
        return {
            "x": _w((lambda *s: _rng.normal(s) * 0.05)(B, S, D)),
            "w1": _w((lambda *s: _rng.normal(s) * 0.05)(D, Dff)),
            "w2": _w((lambda *s: _rng.normal(s) * 0.05)(Dff, D)),
        }
    _B_in = _B_setup()

    return {
        "A_x": _A_in["x"],
        "A_wqkv": _A_in["wqkv"],
        "A_wo": _A_in["wo"],
        "B_x": _B_in["x"],
        "B_w1": _B_in["w1"],
        "B_w2": _B_in["w2"],
        "gate_w": _w((lambda *s: _rng.normal(s) * 0.05)(640) * 16.0),
    }

def reference(A_x, A_wqkv, A_wo, B_x, B_w1, B_w2, gate_w):
    def _A_ref(x, wqkv, wo):
        B, S, D = x.shape
        H = 32; Dh = D // H
        qkv = (lambda x, *d: x.transpose(*d))((x @ wqkv).reshape(B, S, 3, H, Dh), 2, 0, 3, 1, 4)
        q, k, v = qkv[0], qkv[1], qkv[2]
        scale = Dh ** -0.5
        scores = jnp.einsum("bhqd,bhkd->bhqk", q, k) * scale
        p = _softmax(scores, axis=-1)
        o = jnp.einsum("bhqk,bhkd->bhqd", p, v)
        return (lambda x, *d: x.transpose(*d))(o, 0, 2, 1, 3).reshape(B, S, D) @ wo

    def _B_ref(x, w1, w2):
        h = jnp.einsum("bsd,df->bsf", x, w1)
        zero = jnp.zeros_like(h)
        h = jnp.maximum(h, zero)
        return jnp.einsum("bsf,fd->bsd", h, w2)

    x = A_x
    g = _sigmoid((x * gate_w).sum(-1, keepdims=True))
    a = _A_ref(x, A_wqkv, A_wo)
    b = _B_ref(x, B_w1, B_w2)
    return g * a + (1 - g) * b
```

```python
import math

import jax
import jax.numpy as jnp
import jax.experimental.pallas as pl
import jax.experimental.pallas.tpu as pltpu

S = 2048
D = 640
H = 32
DH = 20
DFF = 1536
LANES = 128
NSLAB = D // LANES
TQ = 512
NSUB = S // TQ
CK = 128
NCK = S // CK
TP = 512
TO = 512
QSCALE = (DH ** -0.5) * math.log2(math.e)

_F32 = jnp.float32
_BF16 = jnp.bfloat16


def _kernel(x_ref, wqkv_ref, wo_ref, w1_ref, w2_ref, gw_ref, out_ref,
            kslab, qt, vta, ot, s0, s1, m0, m1):
    def proj(t, carry):
        r0 = pl.multiple_of(t * TP, TP)
        xt = x_ref[pl.ds(r0, TP), :]
        k = jnp.dot(xt, wqkv_ref[:, D:2 * D], preferred_element_type=_F32)
        lane = jax.lax.broadcasted_iota(jnp.int32, (TP, LANES), 1)
        for j in range(NSLAB):
            kj = k[:, j * LANES:(j + 1) * LANES]
            kslab[j, pl.ds(r0, TP), :] = kj.astype(_BF16)
            if j + 1 < NSLAB:
                kn = k[:, (j + 1) * LANES:(j + 2) * LANES]
                kslab[NSLAB + j, pl.ds(r0, TP), :] = jnp.where(
                    lane >= LANES // 2, kj, kn).astype(_BF16)
        tdims = (((0,), (1,)), ((), ()))
        q_t = jax.lax.dot_general(wqkv_ref[:, 0:D], xt, tdims,
                                  preferred_element_type=_F32)
        qt[:, pl.ds(r0, TP)] = (q_t * QSCALE).astype(_BF16)
        v_t = jax.lax.dot_general(wqkv_ref[:, 2 * D:3 * D], xt, tdims,
                                  preferred_element_type=_F32)
        ones = jnp.ones((8, TP), _F32)
        for p in range(H // 2):
            b = 2 * DH * p
            vta[2 * p, :, pl.ds(r0, TP)] = jnp.concatenate(
                [v_t[b:b + 24], ones], axis=0).astype(_BF16)
            vta[2 * p + 1, :, pl.ds(r0, TP)] = jnp.concatenate(
                [v_t[b + 16:b + 40], ones], axis=0).astype(_BF16)
        return carry

    jax.lax.fori_loop(0, S // TP, proj, 0)

    def stage(ha, s_w, m_w, hb, s_r, m_r, b_odd):
        if ha is not None:
            c0 = ha * DH
            j = c0 // LANES
            lo = c0 - j * LANES
            hi2 = lo + DH - LANES
            kidx = jnp.where(hi2 > 0, NSLAB + j, j)
            j2 = jnp.minimum(j + 1, NSLAB - 1)
            row = jax.lax.broadcasted_iota(jnp.int32, (LANES, TQ), 0)
            mask1 = jnp.logical_and(row >= lo, row < lo + DH)
            mask2 = row < hi2
            q1 = pl.multiple_of(j * LANES, LANES)
            q2 = pl.multiple_of(j2 * LANES, LANES)
        if hb is not None:
            pb = hb // 2
        for u in range(NSUB):
            cols = slice(u * TQ, (u + 1) * TQ)
            if ha is not None:
                qa = qt[pl.ds(q1, LANES), cols].astype(_F32)
                qb = qt[pl.ds(q2, LANES), cols].astype(_F32)
                qm = jnp.where(mask1, qa, jnp.where(mask2, qb, 0.0)).astype(_BF16)
                macc = None
            if hb is not None:
                mcur = m_r[u]
                acc = None
            for c in range(NCK):
                rows = slice(c * CK, (c + 1) * CK)
                if ha is not None:
                    s = jnp.dot(kslab[kidx, rows, :], qm,
                                preferred_element_type=_F32)
                    s_w[u, rows, :] = s
                    mc = jnp.max(s.reshape(CK // 8, 8, TQ), axis=0)
                    macc = mc if macc is None else jnp.maximum(macc, mc)
                if hb is not None:
                    sr = s_r[u, rows, :].reshape(CK // 8, 8, TQ)
                    p = jnp.exp2(sr - mcur[None]).reshape(CK, TQ).astype(_BF16)
                    pv = jnp.dot(vta[hb, :, rows], p,
                                 preferred_element_type=_F32)
                    acc = pv if acc is None else acc + pv
            if ha is not None:
                m_w[u] = jnp.broadcast_to(
                    jnp.max(macc, axis=0, keepdims=True), (8, TQ))
            if hb is not None:
                inv = 1.0 / acc[24:25, :]
                if b_odd:
                    ot[pb, DH:2 * DH, cols] = acc[4:24, :] * inv
                else:
                    ot[pb, 0:DH, cols] = acc[0:DH, :] * inv

    stage(0, s0, m0, None, None, None, False)

    def att(i, carry):
        @pl.when(i % 2 == 0)
        def _():
            stage(i + 1, s1, m1, i, s0, m0, False)

        @pl.when(i % 2 == 1)
        def _():
            stage(i + 1, s0, m0, i, s1, m1, True)
        return carry

    jax.lax.fori_loop(0, H - 1, att, 0)
    stage(None, None, None, H - 1, s1, m1, True)

    def outp(t, carry):
        r0 = pl.multiple_of(t * TO, TO)
        xt = x_ref[pl.ds(r0, TO), :]
        o_t = ot[:, :, pl.ds(r0, TO)].reshape(D, TO).astype(_BF16)
        a = jax.lax.dot_general(o_t, wo_ref[...], (((0,), (0,)), ((), ())),
                                preferred_element_type=_F32)
        h = jnp.dot(xt, w1_ref[...], preferred_element_type=_F32)
        h = jnp.maximum(h, 0.0).astype(_BF16)
        b = jnp.dot(h, w2_ref[...], preferred_element_type=_F32)
        z = jnp.sum(xt.astype(_F32) * gw_ref[...].astype(_F32), axis=-1,
                    keepdims=True)
        g = 1.0 / (1.0 + jnp.exp(-z))
        out_ref[pl.ds(r0, TO), :] = (g * a + (1.0 - g) * b).astype(out_ref.dtype)
        return carry

    jax.lax.fori_loop(0, S // TO, outp, 0)


@jax.jit
def pallas_gated_mix__softmax_full_mha__dense_activation_relu__prompt_kernel(
    A_x: jax.Array,
    A_wqkv: jax.Array,
    A_wo: jax.Array,
    B_x: jax.Array,
    B_w1: jax.Array,
    B_w2: jax.Array,
    gate_w: jax.Array,
):
    del B_x
    x = A_x.reshape(S, D)
    gw = gate_w.reshape(1, D)
    out = pl.pallas_call(
        _kernel,
        out_shape=jax.ShapeDtypeStruct((S, D), A_x.dtype),
        scratch_shapes=[
            pltpu.VMEM((2 * NSLAB - 1, S, LANES), _BF16),
            pltpu.VMEM((D, S), _BF16),
            pltpu.VMEM((H, 32, S), _BF16),
            pltpu.VMEM((H // 2, 2 * DH, S), _F32),
            pltpu.VMEM((NSUB, S, TQ), _F32),
            pltpu.VMEM((NSUB, S, TQ), _F32),
            pltpu.VMEM((NSUB, 8, TQ), _F32),
            pltpu.VMEM((NSUB, 8, TQ), _F32),
        ],
        compiler_params=pltpu.CompilerParams(
            vmem_limit_bytes=112 * 1024 * 1024),
    )(x, A_wqkv, A_wo, B_w1, B_w2, gw)
    return out.reshape(A_x.shape)
```

```python
import math

import jax
import jax.numpy as jnp
import jax.experimental.pallas as pl
import jax.experimental.pallas.tpu as pltpu

S = 2048
D = 640
H = 32
DH = 20
DFF = 1536
LANES = 128
NSLAB = D // LANES
TQ = 512
NSUB = S // TQ
CK = 128
NCK = S // CK
TP = 512
NP = S // TP
TO = 512
NO = S // TO
QSCALE = (DH ** -0.5) * math.log2(math.e)

_F32 = jnp.float32
_BF16 = jnp.bfloat16

_SEM_WK, _SEM_WQ, _SEM_WV, _SEM_WO, _SEM_W1, _SEM_W2, _SEM_GW = range(7)
_SEM_X = 7
_SEM_OUT = _SEM_X + NP
_NSEM = _SEM_OUT + NO


def _head_windows(h):
    c0 = h * DH
    j = c0 // LANES
    lo = c0 - j * LANES
    hi = lo + DH
    wins = []
    a = (lo // 16) * 16
    b = min(LANES, -(-hi // 16) * 16)
    wins.append((a, j * LANES + a, b - a, lo - a, min(hi, LANES) - a))
    if hi > LANES:
        n = -(-(hi - LANES) // 16) * 16
        wins.append((0, (j + 1) * LANES, n, 0, hi - LANES))
    return wins


def _kernel(x_hbm, wqkv_hbm, wo_hbm, w1_hbm, w2_hbm, gw_hbm, out_hbm,
            x_v, wqkv_v, wo_v, w1_v, w2_v, gw_v, out_v,
            kslab, qm_all, vta, ot, s0, s1, m0, m1, sems):
    def wcopy(col, slot):
        return pltpu.make_async_copy(
            wqkv_hbm.at[:, pl.ds(col * D, D)], wqkv_v.at[:, pl.ds(col * D, D)],
            sems.at[slot])

    def xcopy(t):
        return pltpu.make_async_copy(
            x_hbm.at[pl.ds(t * TP, TP), :], x_v.at[pl.ds(t * TP, TP), :],
            sems.at[_SEM_X + t])

    def ocopy(t):
        return pltpu.make_async_copy(
            out_v.at[pl.ds(t * TO, TO), :], out_hbm.at[pl.ds(t * TO, TO), :],
            sems.at[_SEM_OUT + t])

    late = [pltpu.make_async_copy(w1_hbm, w1_v, sems.at[_SEM_W1]),
            pltpu.make_async_copy(w2_hbm, w2_v, sems.at[_SEM_W2]),
            pltpu.make_async_copy(wo_hbm, wo_v, sems.at[_SEM_WO]),
            pltpu.make_async_copy(gw_hbm, gw_v, sems.at[_SEM_GW])]

    wcopy(1, _SEM_WK).start()
    xcopy(0).start()
    wcopy(0, _SEM_WQ).start()
    wcopy(2, _SEM_WV).start()

    def zero(h, carry):
        qm_all[h] = jnp.zeros((LANES, S), _BF16)
        return carry
    jax.lax.fori_loop(0, H, zero, 0)

    wcopy(1, _SEM_WK).wait()
    wcopy(0, _SEM_WQ).wait()
    wcopy(2, _SEM_WV).wait()
    for t in range(1, NP):
        xcopy(t).start()

    def proj(t, carry):
        r0 = pl.multiple_of(t * TP, TP)
        pltpu.make_async_copy(
            x_hbm.at[pl.ds(r0, TP), :], x_v.at[pl.ds(r0, TP), :],
            sems.at[_SEM_X + t]).wait()

        @pl.when(t == 1)
        def _():
            for cp in late:
                cp.start()

        xt = x_v[pl.ds(r0, TP), :]
        k = jnp.dot(xt, wqkv_v[:, D:2 * D], preferred_element_type=_F32)
        lane = jax.lax.broadcasted_iota(jnp.int32, (TP, LANES), 1)
        for j in range(NSLAB):
            kj = k[:, j * LANES:(j + 1) * LANES]
            kslab[j, pl.ds(r0, TP), :] = kj.astype(_BF16)
            if j + 1 < NSLAB:
                kn = k[:, (j + 1) * LANES:(j + 2) * LANES]
                kslab[NSLAB + j, pl.ds(r0, TP), :] = jnp.where(
                    lane >= LANES // 2, kj, kn).astype(_BF16)
        tdims = (((0,), (1,)), ((), ()))
        q_t = jax.lax.dot_general(wqkv_v[:, 0:D], xt, tdims,
                                  preferred_element_type=_F32) * QSCALE
        for h in range(H):
            for (dst, src, n, vlo, vhi) in _head_windows(h):
                row = jax.lax.broadcasted_iota(jnp.int32, (n, TP), 0)
                ok = jnp.logical_and(row >= vlo, row < vhi)
                qm_all[h, dst:dst + n, pl.ds(r0, TP)] = jnp.where(
                    ok, q_t[src:src + n], 0.0).astype(_BF16)
        v_t = jax.lax.dot_general(wqkv_v[:, 2 * D:3 * D], xt, tdims,
                                  preferred_element_type=_F32)
        ones = jnp.ones((8, TP), _F32)
        for p in range(H // 2):
            b = 2 * DH * p
            vta[2 * p, :, pl.ds(r0, TP)] = jnp.concatenate(
                [v_t[b:b + 24], ones], axis=0).astype(_BF16)
            vta[2 * p + 1, :, pl.ds(r0, TP)] = jnp.concatenate(
                [v_t[b + 16:b + 40], ones], axis=0).astype(_BF16)
        return carry

    jax.lax.fori_loop(0, NP, proj, 0)

    def stage(ha, s_w, m_w, hb, s_r, m_r, b_odd):
        if ha is not None:
            c0 = ha * DH
            j = c0 // LANES
            straddle = (c0 - j * LANES) + DH > LANES
            kidx = jnp.where(straddle, NSLAB + j, j)
        if hb is not None:
            pb = hb // 2
        for u in range(NSUB):
            cols = slice(u * TQ, (u + 1) * TQ)
            if ha is not None:
                qm = qm_all[ha, :, cols]
                macc = None
            if hb is not None:
                mcur = m_r[u]
                acc = None
            for c in range(NCK):
                rows = slice(c * CK, (c + 1) * CK)
                if ha is not None:
                    s = jnp.dot(kslab[kidx, rows, :], qm,
                                preferred_element_type=_F32)
                    s_w[u, rows, :] = s
                    mc = jnp.max(s.reshape(CK // 8, 8, TQ), axis=0)
                    macc = mc if macc is None else jnp.maximum(macc, mc)
                if hb is not None:
                    sr = s_r[u, rows, :].reshape(CK // 8, 8, TQ)
                    p = jnp.exp2(sr - mcur[None]).reshape(CK, TQ).astype(_BF16)
                    pv = jnp.dot(vta[hb, :, rows], p,
                                 preferred_element_type=_F32)
                    acc = pv if acc is None else acc + pv
            if ha is not None:
                m_w[u] = jnp.broadcast_to(
                    jnp.max(macc, axis=0, keepdims=True), (8, TQ))
            if hb is not None:
                inv = 1.0 / acc[24:25, :]
                if b_odd:
                    ot[pb, DH:2 * DH, cols] = acc[4:24, :] * inv
                else:
                    ot[pb, 0:DH, cols] = acc[0:DH, :] * inv

    stage(0, s0, m0, None, None, None, False)

    def att(i, carry):
        @pl.when(i % 2 == 0)
        def _():
            stage(i + 1, s1, m1, i, s0, m0, False)

        @pl.when(i % 2 == 1)
        def _():
            stage(i + 1, s0, m0, i, s1, m1, True)
        return carry

    jax.lax.fori_loop(0, H - 1, att, 0)
    stage(None, None, None, H - 1, s1, m1, True)

    for cp in late:
        cp.wait()

    def outp(t, carry):
        r0 = pl.multiple_of(t * TO, TO)
        xt = x_v[pl.ds(r0, TO), :]
        o_t = ot[:, :, pl.ds(r0, TO)].reshape(D, TO).astype(_BF16)
        a = jax.lax.dot_general(o_t, wo_v[...], (((0,), (0,)), ((), ())),
                                preferred_element_type=_F32)
        h = jnp.dot(xt, w1_v[...], preferred_element_type=_F32)
        h = jnp.maximum(h, 0.0).astype(_BF16)
        b = jnp.dot(h, w2_v[...], preferred_element_type=_F32)
        gw = gw_v[...].astype(_F32).reshape(1, D)
        z = jnp.sum(xt.astype(_F32) * gw, axis=-1, keepdims=True)
        g = 1.0 / (1.0 + jnp.exp(-z))
        out_v[pl.ds(r0, TO), :] = (g * a + (1.0 - g) * b).astype(out_v.dtype)
        pltpu.make_async_copy(
            out_v.at[pl.ds(r0, TO), :], out_hbm.at[pl.ds(r0, TO), :],
            sems.at[_SEM_OUT + t]).start()
        return carry

    jax.lax.fori_loop(0, NO, outp, 0)
    for t in range(NO):
        ocopy(t).wait()


@jax.jit
def pallas_gated_mix__softmax_full_mha__dense_activation_relu__prompt_kernel(
    A_x: jax.Array,
    A_wqkv: jax.Array,
    A_wo: jax.Array,
    B_x: jax.Array,
    B_w1: jax.Array,
    B_w2: jax.Array,
    gate_w: jax.Array,
):
    del B_x
    x = A_x.reshape(S, D)
    any_spec = pl.BlockSpec(memory_space=pl.ANY)
    out = pl.pallas_call(
        _kernel,
        out_shape=jax.ShapeDtypeStruct((S, D), A_x.dtype),
        in_specs=[any_spec] * 6,
        out_specs=any_spec,
        scratch_shapes=[
            pltpu.VMEM((S, D), _BF16),
            pltpu.VMEM((D, 3 * D), _BF16),
            pltpu.VMEM((D, D), _BF16),
            pltpu.VMEM((D, DFF), _BF16),
            pltpu.VMEM((DFF, D), _BF16),
            pltpu.VMEM((D,), _BF16),
            pltpu.VMEM((S, D), _BF16),
            pltpu.VMEM((2 * NSLAB - 1, S, LANES), _BF16),
            pltpu.VMEM((H, LANES, S), _BF16),
            pltpu.VMEM((H, 32, S), _BF16),
            pltpu.VMEM((H // 2, 2 * DH, S), _F32),
            pltpu.VMEM((NSUB, S, TQ), _F32),
            pltpu.VMEM((NSUB, S, TQ), _F32),
            pltpu.VMEM((NSUB, 8, TQ), _F32),
            pltpu.VMEM((NSUB, 8, TQ), _F32),
            pltpu.SemaphoreType.DMA((_NSEM,)),
        ],
        compiler_params=pltpu.CompilerParams(
            vmem_limit_bytes=120 * 1024 * 1024),
    )(x, A_wqkv, A_wo, B_w1, B_w2, gate_w)
    return out.reshape(A_x.shape)
```

```python
import math

import jax
import jax.numpy as jnp
import jax.experimental.pallas as pl
import jax.experimental.pallas.tpu as pltpu

S = 2048
D = 640
H = 32
DH = 20
DFF = 1536
LANES = 128
NSLAB = D // LANES
TQ = 128
NSUB = S // TQ
NT = TQ // LANES
NV = 176
NG = 2
NMR = S - NV
CK = 128
NCK = S // CK
TP = 512
NP = S // TP
TO = 512
NO = S // TO
QSCALE = (DH ** -0.5) * math.log2(math.e)

_F32 = jnp.float32
_BF16 = jnp.bfloat16
_U32 = jnp.uint32


def _pack(x):
    return pltpu.bitcast(x.astype(_BF16), _U32)


def _unpack(x):
    return pltpu.bitcast(x, _BF16)

_SEM_WK, _SEM_WQ, _SEM_WV, _SEM_WO, _SEM_W1, _SEM_W2, _SEM_GW = range(7)
_SEM_X = 7
_SEM_OUT = _SEM_X + NP
_NSEM = _SEM_OUT + NO


def _head_windows(h):
    c0 = h * DH
    j = c0 // LANES
    lo = c0 - j * LANES
    hi = lo + DH
    wins = []
    a = (lo // 16) * 16
    b = min(LANES, -(-hi // 16) * 16)
    wins.append((a, j * LANES + a, b - a, lo - a, min(hi, LANES) - a))
    if hi > LANES:
        n = -(-(hi - LANES) // 16) * 16
        wins.append((0, (j + 1) * LANES, n, 0, hi - LANES))
    return wins


def _kernel(x_hbm, wqkv_hbm, wo_hbm, w1_hbm, w2_hbm, gw_hbm, out_hbm,
            x_v, wqkv_v, wo_v, w1_v, w2_v, gw_v, out_v,
            kslab, qm_all, qh32, vta, ot, s0, s1, m0, m1,
            kb0, kb1, qb0, qb1, zero_s, sems):
    def wcopy(col, slot):
        return pltpu.make_async_copy(
            wqkv_hbm.at[:, pl.ds(col * D, D)], wqkv_v.at[:, pl.ds(col * D, D)],
            sems.at[slot])

    def xcopy(t):
        return pltpu.make_async_copy(
            x_hbm.at[pl.ds(t * TP, TP), :], x_v.at[pl.ds(t * TP, TP), :],
            sems.at[_SEM_X + t])

    def ocopy(t):
        return pltpu.make_async_copy(
            out_v.at[pl.ds(t * TO, TO), :], out_hbm.at[pl.ds(t * TO, TO), :],
            sems.at[_SEM_OUT + t])

    late = [pltpu.make_async_copy(w1_hbm, w1_v, sems.at[_SEM_W1]),
            pltpu.make_async_copy(w2_hbm, w2_v, sems.at[_SEM_W2]),
            pltpu.make_async_copy(wo_hbm, wo_v, sems.at[_SEM_WO]),
            pltpu.make_async_copy(gw_hbm, gw_v, sems.at[_SEM_GW])]

    zero_s[0] = 0
    wcopy(1, _SEM_WK).start()
    xcopy(0).start()
    wcopy(0, _SEM_WQ).start()
    wcopy(2, _SEM_WV).start()

    def zero(h, carry):
        qm_all[h] = jnp.zeros((LANES // 2, S), _U32)
        return carry
    jax.lax.fori_loop(0, H, zero, 0)

    wcopy(1, _SEM_WK).wait()
    wcopy(0, _SEM_WQ).wait()
    wcopy(2, _SEM_WV).wait()
    for t in range(1, NP):
        xcopy(t).start()

    def proj(t, carry):
        r0 = pl.multiple_of(t * TP, TP)
        pltpu.make_async_copy(
            x_hbm.at[pl.ds(r0, TP), :], x_v.at[pl.ds(r0, TP), :],
            sems.at[_SEM_X + t]).wait()

        @pl.when(t == 1)
        def _():
            for cp in late:
                cp.start()

        rh = pl.multiple_of(t * (TP // 2), TP // 2)
        xt = x_v[pl.ds(r0, TP), :]
        k = jnp.dot(xt, wqkv_v[:, D:2 * D], preferred_element_type=_F32)
        lane = jax.lax.broadcasted_iota(jnp.int32, (TP, LANES), 1)
        for j in range(NSLAB):
            kj = k[:, j * LANES:(j + 1) * LANES]
            kslab[j, pl.ds(rh, TP // 2), :] = _pack(kj)
            if j + 1 < NSLAB:
                kn = k[:, (j + 1) * LANES:(j + 2) * LANES]
                kslab[NSLAB + j, pl.ds(rh, TP // 2), :] = _pack(jnp.where(
                    lane >= LANES // 2, kj, kn))
        tdims = (((0,), (1,)), ((), ()))
        q_t = jax.lax.dot_general(wqkv_v[:, 0:D], xt, tdims,
                                  preferred_element_type=_F32) * QSCALE
        qh32[:, :, pl.ds(r0, TP)] = q_t.astype(_BF16).astype(_F32).reshape(
            H // 2, 2 * DH, TP)
        for h in range(H):
            for (dst, src, n, vlo, vhi) in _head_windows(h):
                row = jax.lax.broadcasted_iota(jnp.int32, (n, TP), 0)
                ok = jnp.logical_and(row >= vlo, row < vhi)
                qm_all[h, dst // 2:(dst + n) // 2, pl.ds(r0, TP)] = _pack(
                    jnp.where(ok, q_t[src:src + n], 0.0))
        v_t = jax.lax.dot_general(wqkv_v[:, 2 * D:3 * D], xt, tdims,
                                  preferred_element_type=_F32)
        ones = jnp.ones((8, TP), _F32)
        for p in range(H // 2):
            b = 2 * DH * p
            vta[2 * p, :, pl.ds(r0, TP)] = _pack(jnp.concatenate(
                [v_t[b:b + 24], ones], axis=0))
            vta[2 * p + 1, :, pl.ds(r0, TP)] = _pack(jnp.concatenate(
                [v_t[b + 16:b + 40], ones], axis=0))
        return carry

    jax.lax.fori_loop(0, NP, proj, 0)

    def slab_of(h):
        c0 = h * DH
        j = c0 // LANES
        lo = c0 - j * LANES
        return jnp.where(lo + DH > LANES, NSLAB + j, j), lo

    def stage(a, b, c):
        use_vpu = a is not None and a[3] is not None
        nmr = NMR if use_vpu else S
        nrg = nmr // 8
        npiece = NV // (8 * NG) if use_vpu else 0
        if a is not None:
            ha, s_w, m_w, kb_r, qb_r = a
            kidx, _ = slab_of(ha)
        if b is not None:
            hb, b_odd, s_r, m_r = b
            pb = hb // 2
        prep = []
        if c is not None:
            hc, c_odd, kb_w, qb_w = c
            zmask = jnp.full((8, LANES), zero_s[0], jnp.int32)
            cidx, clo = slab_of(hc)
            kv = pltpu.roll(_unpack(kslab[cidx, NMR // 2:S // 2, :]).astype(_F32),
                            (LANES - clo) % LANES, 1)
            w0 = 16 if c_odd else 0
            woff = 4 if c_odd else 0

            def gate(x, zero):
                n = x.shape[0] // 8
                z = jnp.concatenate([zero] * n, axis=0) if n > 1 else zero
                return pltpu.bitcast(pltpu.bitcast(x, jnp.int32) | z, _F32)

            def prep_k(d, zero):
                kb_w[d] = jnp.broadcast_to(gate(kv, zero)[:, d:d + 1],
                                           (NV, LANES))

            def prep_q(t, zero):
                lanes = slice(t * LANES, (t + 1) * LANES)
                win = gate(qh32[hc // 2, w0:w0 + 24, lanes], zero)
                for d in range(DH):
                    qb_w[d, :, lanes] = jnp.broadcast_to(
                        win[woff + d:woff + d + 1, :], (8, LANES))

            ks = [(prep_k, d) for d in range(DH)]
            qs = [(prep_q, t) for t in range(S // LANES)]
            while ks or qs:
                if ks:
                    prep.append(ks.pop(0))
                if qs:
                    prep.append(qs.pop(0))
        nprep = len(prep)
        tot_rg = NSUB * nrg
        pi = 0
        for u in range(NSUB):
            cols = slice(u * TQ, (u + 1) * TQ)
            if a is not None:
                qm = _unpack(qm_all[ha, :, cols])
                macc = [None] * NT

                def piece(w, u=u, macc=macc):
                    sv = {}
                    for d in range(DH):
                        qd = [qb_r[d, :, u * TQ + t * LANES:u * TQ + (t + 1) * LANES]
                              for t in range(NT)]
                        for g in range(w * NG, (w + 1) * NG):
                            kb = kb_r[d, g * 8:(g + 1) * 8, :]
                            for t in range(NT):
                                pr = kb * qd[t]
                                sv[(g, t)] = pr if d == 0 else sv[(g, t)] + pr
                    for (g, t), v in sv.items():
                        s_w[u, NMR + g * 8:NMR + (g + 1) * 8,
                            t * LANES:(t + 1) * LANES] = v
                        macc[t] = jnp.maximum(macc[t], v)
            if b is not None:
                mcur = m_r[u]
                acc = None
            wi = 0
            ra = 0
            for ci in range(NCK):
                rows = slice(ci * CK, (ci + 1) * CK)
                if a is not None and ci * CK < nmr:
                    r0, r1 = ci * CK, min((ci + 1) * CK, nmr)
                    s = jnp.dot(_unpack(kslab[kidx, r0 // 2:r1 // 2, :]), qm,
                                preferred_element_type=_F32)
                    s_w[u, r0:r1, :] = s
                    for rg in range((r1 - r0) // 8):
                        for t in range(NT):
                            v = s[rg * 8:(rg + 1) * 8, t * LANES:(t + 1) * LANES]
                            macc[t] = v if macc[t] is None else jnp.maximum(macc[t], v)
                        ra += 1
                        while wi < npiece and wi * nrg < ra * npiece - nrg // 2:
                            piece(wi)
                            wi += 1
                        while (pi < nprep and
                               (pi + 1) * tot_rg <= (u * nrg + ra) * (nprep + 2)):
                            fn, arg = prep[pi]
                            fn(arg, pltpu.bitcast(v, jnp.int32) & zmask)
                            pi += 1
                if b is not None:
                    sr = s_r[u, rows, :].reshape(CK // 8, 8, TQ)
                    p = jnp.exp2(sr - mcur[None]).reshape(CK, TQ).astype(_BF16)
                    pv = jnp.dot(_unpack(vta[hb, :, rows]), p,
                                 preferred_element_type=_F32)
                    acc = pv if acc is None else acc + pv
            if a is not None:
                while wi < npiece:
                    piece(wi)
                    wi += 1
                m_w[u] = jnp.broadcast_to(
                    jnp.max(jnp.concatenate(macc, axis=1), axis=0,
                            keepdims=True), (8, TQ))
            if b is not None:
                inv = 1.0 / acc[24:25, :]
                if b_odd:
                    ot[pb, DH:2 * DH, cols] = acc[4:24, :] * inv
                else:
                    ot[pb, 0:DH, cols] = acc[0:DH, :] * inv
        assert pi == nprep

    stage((0, s0, m0, None, None), None, (1, True, kb1, qb1))

    def att(i, carry):
        @pl.when(i % 2 == 0)
        def _():
            hc = jnp.minimum(i + 2, H - 2)
            stage((i + 1, s1, m1, kb1, qb1), (i, False, s0, m0),
                  (hc, False, kb0, qb0))

        @pl.when(i % 2 == 1)
        def _():
            stage((i + 1, s0, m0, kb0, qb0), (i, True, s1, m1),
                  (i + 2, True, kb1, qb1))
        return carry

    jax.lax.fori_loop(0, H - 1, att, 0)
    stage(None, (H - 1, True, s1, m1), None)

    for cp in late:
        cp.wait()

    def outp(t, carry):
        r0 = pl.multiple_of(t * TO, TO)
        xt = x_v[pl.ds(r0, TO), :]
        o_t = ot[:, :, pl.ds(r0, TO)].reshape(D, TO).astype(_BF16)
        a = jax.lax.dot_general(o_t, wo_v[...], (((0,), (0,)), ((), ())),
                                preferred_element_type=_F32)
        h = jnp.dot(xt, w1_v[...], preferred_element_type=_F32)
        h = jnp.maximum(h, 0.0).astype(_BF16)
        b = jnp.dot(h, w2_v[...], preferred_element_type=_F32)
        gw = gw_v[...].astype(_F32).reshape(1, D)
        z = jnp.sum(xt.astype(_F32) * gw, axis=-1, keepdims=True)
        g = 1.0 / (1.0 + jnp.exp(-z))
        out_v[pl.ds(r0, TO), :] = (g * a + (1.0 - g) * b).astype(out_v.dtype)
        pltpu.make_async_copy(
            out_v.at[pl.ds(r0, TO), :], out_hbm.at[pl.ds(r0, TO), :],
            sems.at[_SEM_OUT + t]).start()
        return carry

    jax.lax.fori_loop(0, NO, outp, 0)
    for t in range(NO):
        ocopy(t).wait()


@jax.jit
def pallas_gated_mix__softmax_full_mha__dense_activation_relu__prompt_kernel(
    A_x: jax.Array,
    A_wqkv: jax.Array,
    A_wo: jax.Array,
    B_x: jax.Array,
    B_w1: jax.Array,
    B_w2: jax.Array,
    gate_w: jax.Array,
):
    del B_x
    x = A_x.reshape(S, D)
    any_spec = pl.BlockSpec(memory_space=pl.ANY)
    out = pl.pallas_call(
        _kernel,
        out_shape=jax.ShapeDtypeStruct((S, D), A_x.dtype),
        in_specs=[any_spec] * 6,
        out_specs=any_spec,
        scratch_shapes=[
            pltpu.VMEM((S, D), _BF16),
            pltpu.VMEM((D, 3 * D), _BF16),
            pltpu.VMEM((D, D), _BF16),
            pltpu.VMEM((D, DFF), _BF16),
            pltpu.VMEM((DFF, D), _BF16),
            pltpu.VMEM((D,), _BF16),
            pltpu.VMEM((S, D), _BF16),
            pltpu.VMEM((2 * NSLAB - 1, S // 2, LANES), _U32),
            pltpu.VMEM((H, LANES // 2, S), _U32),
            pltpu.VMEM((H // 2, 2 * DH, S), _F32),
            pltpu.VMEM((H, 16, S), _U32),
            pltpu.VMEM((H // 2, 2 * DH, S), _F32),
            pltpu.VMEM((NSUB, S, TQ), _F32),
            pltpu.VMEM((NSUB, S, TQ), _F32),
            pltpu.VMEM((NSUB, 8, TQ), _F32),
            pltpu.VMEM((NSUB, 8, TQ), _F32),
            pltpu.VMEM((DH, NV, LANES), _F32),
            pltpu.VMEM((DH, NV, LANES), _F32),
            pltpu.VMEM((DH, 8, S), _F32),
            pltpu.VMEM((DH, 8, S), _F32),
            pltpu.SMEM((1,), jnp.int32),
            pltpu.SemaphoreType.DMA((_NSEM,)),
        ],
        compiler_params=pltpu.CompilerParams(
            vmem_limit_bytes=120 * 1024 * 1024),
    )(x, A_wqkv, A_wo, B_w1, B_w2, gate_w)
    return out.reshape(A_x.shape)
```

```python
import math

import jax
import jax.numpy as jnp
import jax.experimental.pallas as pl
import jax.experimental.pallas.tpu as pltpu

S = 2048
D = 640
H = 32
DH = 20
DFF = 1536
LANES = 128
NSLAB = D // LANES
NFT = DFF // LANES
TQ = 128
NSUB = S // TQ
NV = 192
NG = 2
NMR = S - NV
CK = 128
NCK = S // CK
TF = S // H
TP = 512
NP = S // TP
TPQ = 1024
TO = 512
NO = S // TO
QSCALE = (DH ** -0.5) * math.log2(math.e)

_F32 = jnp.float32
_BF16 = jnp.bfloat16
_U32 = jnp.uint32

_SEM_WK, _SEM_WQ, _SEM_WV, _SEM_WO, _SEM_W1, _SEM_W2, _SEM_GW = range(7)
_SEM_X = 7
_SEM_OUT = _SEM_X + NP
_NSEM = _SEM_OUT + NO


def _pack(x):
    return pltpu.bitcast(x.astype(_BF16), _U32)


def _unpack(x):
    return pltpu.bitcast(x, _BF16)


def _head_windows(h):
    c0 = h * DH
    j = c0 // LANES
    lo = c0 - j * LANES
    hi = lo + DH
    a = (lo // 16) * 16
    b = min(LANES, -(-hi // 16) * 16)
    wins = [(a, j * LANES + a, b - a, lo - a, min(hi, LANES) - a)]
    if hi > LANES:
        n = -(-(hi - LANES) // 16) * 16
        wins.append((0, (j + 1) * LANES, n, 0, hi - LANES))
    return wins


def _kernel(x_hbm, wqkv_hbm, wo_hbm, w1_hbm, w2_hbm, gw_hbm, out_hbm,
            x_v, wqkv_v, wo_v, w1_v, w2_v, gw_v, out_v,
            kslab, qm_all, qh32, vta, ot, s0, s1, m0, m1,
            kb0, kb1, qb0, qb1, w1p, w2p, h0, h1, bbuf, gcol, zero_s, sems):
    def wcopy(col, slot):
        dst = (0, 2, 1)[col]
        return pltpu.make_async_copy(
            wqkv_hbm.at[:, pl.ds(col * D, D)], wqkv_v.at[:, pl.ds(dst * D, D)],
            sems.at[slot])

    def gate(x, zero):
        z = jnp.tile(zero, (x.shape[0] // 8, x.shape[1] // LANES))
        return pltpu.bitcast(pltpu.bitcast(x, jnp.int32) | z, x.dtype)

    def zero_of(v):
        zmask = jnp.full((8, LANES), zero_s[0], jnp.int32)
        return pltpu.bitcast(v, jnp.int32) & zmask

    def xcopy(t):
        r0 = pl.multiple_of(t * TP, TP)
        return pltpu.make_async_copy(
            x_hbm.at[pl.ds(r0, TP), :], x_v.at[pl.ds(r0, TP), :],
            sems.at[_SEM_X + t])

    def ocopy(t):
        r0 = pl.multiple_of(t * TO, TO)
        return pltpu.make_async_copy(
            out_v.at[pl.ds(r0, TO), :], out_hbm.at[pl.ds(r0, TO), :],
            sems.at[_SEM_OUT + t])

    late = [pltpu.make_async_copy(w1_hbm, w1_v, sems.at[_SEM_W1]),
            pltpu.make_async_copy(w2_hbm, w2_v, sems.at[_SEM_W2]),
            pltpu.make_async_copy(wo_hbm, wo_v, sems.at[_SEM_WO])]
    gwcopy = pltpu.make_async_copy(gw_hbm, gw_v, sems.at[_SEM_GW])

    zero_s[0] = 0
    gwcopy.start()
    wcopy(1, _SEM_WK).start()
    xcopy(0).start()
    xcopy(1).start()

    def zero(h, carry):
        qm_all[h] = jnp.zeros((LANES // 2, S), _U32)
        return carry
    jax.lax.fori_loop(0, H, zero, 0)

    gwcopy.wait()
    wcopy(1, _SEM_WK).wait()
    xcopy(2).start()
    xcopy(3).start()
    wcopy(0, _SEM_WQ).start()
    wcopy(2, _SEM_WV).start()

    def proj_k(t, carry):
        xcopy(t).wait()
        r0 = pl.multiple_of(t * TP, TP)
        rh = pl.multiple_of(t * (TP // 2), TP // 2)
        xt = x_v[pl.ds(r0, TP), :]
        k = jnp.dot(xt, wqkv_v[:, 2 * D:3 * D], preferred_element_type=_F32)
        gw = jnp.broadcast_to(gw_v[...].astype(_F32).reshape(1, D), (8, D))
        nch = NSLAB - 1
        tc = TP // nch
        for j in range(nch):
            gwj = gate(gw, zero_of(k[0:8, j * LANES:(j + 1) * LANES]))
            xj = xt[j * tc:(j + 1) * tc].astype(_F32).reshape(tc // 8, 8, D)
            z = jnp.sum((xj * gwj[None]).reshape(tc, D), axis=-1, keepdims=True)
            gcol[pl.ds(r0 + j * tc, tc), :] = jnp.broadcast_to(
                1.0 / (1.0 + jnp.exp(-z)), (tc, LANES))
        lane = jax.lax.broadcasted_iota(jnp.int32, (TP, LANES), 1)
        for j in range(NSLAB):
            kj = k[:, j * LANES:(j + 1) * LANES]
            kslab[j, pl.ds(rh, TP // 2), :] = _pack(kj)
            if j + 1 < NSLAB:
                kn = k[:, (j + 1) * LANES:(j + 2) * LANES]
                kslab[NSLAB + j, pl.ds(rh, TP // 2), :] = _pack(jnp.where(
                    lane >= LANES // 2, kj, kn))
        return carry

    jax.lax.fori_loop(0, NP, proj_k, 0)

    wcopy(0, _SEM_WQ).wait()
    wcopy(2, _SEM_WV).wait()
    for cp in late:
        cp.start()

    def proj_qv(t, carry):
        cols = pl.ds(pl.multiple_of(t * TPQ, TPQ), TPQ)
        xt = x_v[cols, :]
        tdims = (((0,), (1,)), ((), ()))
        qv_t = jax.lax.dot_general(wqkv_v[:, 0:2 * D], xt, tdims,
                                   preferred_element_type=_F32)
        q_t = qv_t[0:D] * QSCALE
        v_t = qv_t[D:2 * D]
        qh32[:, :, cols] = q_t.astype(_BF16).astype(_F32).reshape(
            H // 2, 2 * DH, TPQ)
        for h in range(H):
            for (dst, src, n, vlo, vhi) in _head_windows(h):
                row = jax.lax.broadcasted_iota(jnp.int32, (n, TPQ), 0)
                ok = jnp.logical_and(row >= vlo, row < vhi)
                qm_all[h, dst // 2:(dst + n) // 2, cols] = _pack(
                    jnp.where(ok, q_t[src:src + n], 0.0))
        ones = jnp.ones((8, TPQ), _F32)
        for p in range(H // 2):
            b = 2 * DH * p
            vta[2 * p, :, cols] = _pack(jnp.concatenate(
                [v_t[b:b + 24], ones], axis=0))
            vta[2 * p + 1, :, cols] = _pack(jnp.concatenate(
                [v_t[b + 16:b + 40], ones], axis=0))
        return carry

    jax.lax.fori_loop(0, S // TPQ, proj_qv, 0)

    def slab_of(h):
        c0 = h * DH
        j = c0 // LANES
        lo = c0 - j * LANES
        return jnp.where(lo + DH > LANES, NSLAB + j, j), lo

    def ffn_steps(f1, f2, first):
        facc = [None]

        def step(lhs, w, last):
            def run():
                pr = jnp.dot(lhs(), w(), preferred_element_type=_F32)
                facc[0] = pr if facc[0] is None else facc[0] + pr
                if last is not None:
                    last(facc[0])
                    facc[0] = None
            return run

        g1, g2 = [], []
        if f1 is not None:
            f1r = pl.multiple_of(f1[0] * TF, TF)
            for n in range(NFT):
                lanes = slice(n * LANES, (n + 1) * LANES)

                def fin1(hh, lanes=lanes):
                    f1[1][:, lanes] = _pack(jnp.maximum(hh, 0.0))

                def w1_tile(kt, lanes=lanes):
                    if first:
                        return w1_v[kt * LANES:(kt + 1) * LANES, lanes]
                    return _unpack(w1p[kt * 64:(kt + 1) * 64, lanes])
                g1.append([step(
                    lambda kt=kt: x_v[pl.ds(f1r, TF), kt * LANES:(kt + 1) * LANES],
                    lambda kt=kt, w1_tile=w1_tile: w1_tile(kt),
                    fin1 if kt == NSLAB - 1 else None) for kt in range(NSLAB)])
        if f2 is not None:
            f2r = pl.multiple_of(f2[0] * TF, TF)
            for n in range(NSLAB):
                lanes = slice(n * LANES, (n + 1) * LANES)

                def fin2(bb, lanes=lanes):
                    bbuf[pl.ds(f2r, TF), lanes] = bb
                g2.append([step(
                    lambda kt=kt: _unpack(f2[1][:, kt * LANES:(kt + 1) * LANES]),
                    lambda kt=kt, lanes=lanes: _unpack(
                        w2p[kt * 64:(kt + 1) * 64, lanes]),
                    fin2 if kt == NFT - 1 else None) for kt in range(NFT)])
        steps = []
        while g1 or g2:
            n1 = 3 if len(g2) < 3 else 2
            for grp in g1[:2] + g2[:1] + g1[2:n1]:
                steps += grp
            g1, g2 = g1[n1:], g2[1:]
        return steps

    def stage(a, b, c, steps, subs=range(NSUB), ubase=None, repack=False):
        use_vpu = a is not None and a[3] is not None
        nmr = NMR if use_vpu else S
        nrg = nmr // 8
        npiece = NV // (8 * NG) if use_vpu else 0
        if a is not None:
            ha, s_w, m_w, kb_r, qb_r = a
            kidx, _ = slab_of(ha)
        if b is not None:
            hb, b_odd, s_r, m_r = b
        prep = []
        if c is not None:
            hc, c_odd, kb_w, qb_w = c
            cidx, clo = slab_of(hc)
            kv = pltpu.roll(
                _unpack(kslab[cidx, NMR // 2:S // 2, :]).astype(_F32),
                (LANES - clo) % LANES, 1)
            w0 = 16 if c_odd else 0
            woff = 4 if c_odd else 0

            def prep_k(d, zero):
                kb_w[d] = jnp.broadcast_to(gate(kv, zero)[:, d:d + 1],
                                           (NV, LANES))

            def prep_q(t, zero):
                lanes = slice(t * LANES, (t + 1) * LANES)
                win = gate(qh32[hc // 2, w0:w0 + 24, lanes], zero)
                for d in range(DH):
                    qb_w[d, :, lanes] = jnp.broadcast_to(
                        win[woff + d:woff + d + 1, :], (8, LANES))

            def prep_w(nj, zero):
                n, j = nj
                a_ = slice(n * LANES, (n + 1) * LANES)
                b_ = slice(j * LANES, (j + 1) * LANES)
                w2p[n * 64:(n + 1) * 64, b_] = gate(
                    pltpu.bitcast(w2_v[a_, b_], _U32), zero)
                w1p[j * 64:(j + 1) * 64, a_] = gate(
                    pltpu.bitcast(w1_v[b_, a_], _U32), zero)

            lists = [[(prep_k, d) for d in range(DH)],
                     [(prep_q, t) for t in range(S // LANES)]]
            if repack:
                for j0 in range(3):
                    lists.append([(prep_w, (n, j)) for n in range(NFT)
                                  for j in range(NSLAB)][j0::3])
            while any(lists):
                for lst in lists:
                    if lst:
                        prep.append(lst.pop(0))
        nprep = len(prep)
        nsub = len(subs)
        pi = 0
        ui = 0
        for un, u in enumerate(subs):
            if ubase is None:
                cols = slice(u * TQ, (u + 1) * TQ)
            else:
                u = ubase + u
                cols = pl.ds(pl.multiple_of(u * TQ, TQ), TQ)
            if a is not None:
                qm = _unpack(qm_all[ha, :, cols])
                macc = [None]

                def piece(w, u=u, cols=cols, macc=macc):
                    gs = range(w * NG, (w + 1) * NG)
                    sv = {}
                    for d in range(DH):
                        qd = qb_r[d, :, cols]
                        for g in gs:
                            pr = kb_r[d, g * 8:(g + 1) * 8, :] * qd
                            sv[g] = pr if d == 0 else sv[g] + pr
                    for g in gs:
                        s_w[u, NMR + g * 8:NMR + (g + 1) * 8, :] = sv[g]
                        macc[0] = jnp.maximum(macc[0], sv[g])
            if b is not None:
                mcur = m_r[u]
                acc = None
            wi = 0
            ra = 0
            for ci in range(NCK):
                rows = slice(ci * CK, (ci + 1) * CK)
                if a is not None and ci * CK < nmr:
                    r0, r1 = ci * CK, min((ci + 1) * CK, nmr)
                    s = jnp.dot(_unpack(kslab[kidx, r0 // 2:r1 // 2, :]), qm,
                                preferred_element_type=_F32)
                    s_w[u, r0:r1, :] = s
                    for rg in range((r1 - r0) // 8):
                        v = s[rg * 8:(rg + 1) * 8, :]
                        macc[0] = v if macc[0] is None else jnp.maximum(macc[0], v)
                        ra += 1
                        while wi < npiece and wi * nrg < ra * npiece - nrg // 2:
                            piece(wi)
                            wi += 1
                        while (pi < nprep and (pi + 1) * nsub * nrg
                               <= (un * nrg + ra) * (nprep + 2)):
                            fn, arg = prep[pi]
                            fn(arg, zero_of(v))
                            pi += 1
                if b is not None:
                    sr = s_r[u, rows, :].reshape(CK // 8, 8, TQ)
                    p = jnp.exp2(sr - mcur[None]).reshape(CK, TQ).astype(_BF16)
                    pv = jnp.dot(_unpack(vta[hb, :, rows]), p,
                                 preferred_element_type=_F32)
                    acc = pv if acc is None else acc + pv
                while (ui < len(steps) and (ui + 1) * nsub * NCK
                       <= (un * NCK + ci + 2) * len(steps)):
                    steps[ui]()
                    ui += 1
            if a is not None:
                while wi < npiece:
                    piece(wi)
                    wi += 1
                m_w[u] = jnp.broadcast_to(
                    jnp.max(macc[0], axis=0, keepdims=True), (8, TQ))
            if b is not None:
                inv = 1.0 / acc[24:25, :]
                if b_odd:
                    ot[hb // 2, DH:2 * DH, cols] = acc[4:24, :] * inv
                else:
                    ot[hb // 2, 0:DH, cols] = acc[0:DH, :] * inv
        assert pi == nprep and ui == len(steps)

    late[0].wait()
    late[1].wait()
    stage((0, s0, m0, None, None), None, (1, True, kb1, qb1),
          ffn_steps((0, h0), None, True), repack=True)

    def att(i, carry):
        @pl.when(i % 2 == 0)
        def _():
            hc = jnp.minimum(i + 2, H - 2)
            stage((i + 1, s1, m1, kb1, qb1), (i, False, s0, m0),
                  (hc, False, kb0, qb0), ffn_steps((i + 1, h1), (i, h0), False))

        @pl.when(i % 2 == 1)
        def _():
            stage((i + 1, s0, m0, kb0, qb0), (i, True, s1, m1),
                  (i + 2, True, kb1, qb1), ffn_steps((i + 1, h0), (i, h1), False))
        return carry

    jax.lax.fori_loop(0, H - 1, att, 0)

    spt = TO // TQ
    last_b = (H - 1, True, s1, m1)
    stage(None, last_b, None, ffn_steps(None, (H - 1, h1), False),
          subs=range(spt))
    late[2].wait()

    def out_steps(t):
        r0 = pl.multiple_of(t * TO, TO)
        rows = pl.ds(r0, TO)
        o_t = ot[:, :, rows].reshape(D, TO).astype(_BF16)

        def step(n):
            def run():
                lanes = slice(n * LANES, (n + 1) * LANES)
                g = gcol[rows, :]
                a = jax.lax.dot_general(o_t, wo_v[:, lanes],
                                        (((0,), (0,)), ((), ())),
                                        preferred_element_type=_F32)
                out_v[rows, lanes] = (
                    g * a + (1.0 - g) * bbuf[rows, lanes]).astype(out_v.dtype)
            return run
        return [step(n) for n in range(NSLAB)]

    def outp(t, carry):
        stage(None, last_b, None, out_steps(t), subs=range(spt),
              ubase=(t + 1) * spt)
        ocopy(t).start()
        return carry

    jax.lax.fori_loop(0, NO - 1, outp, 0)
    for run in out_steps(NO - 1):
        run()
    ocopy(NO - 1).start()
    for t in range(NO):
        ocopy(t).wait()


@jax.jit
def pallas_gated_mix__softmax_full_mha__dense_activation_relu__prompt_kernel(
    A_x: jax.Array,
    A_wqkv: jax.Array,
    A_wo: jax.Array,
    B_x: jax.Array,
    B_w1: jax.Array,
    B_w2: jax.Array,
    gate_w: jax.Array,
):
    del B_x
    x = A_x.reshape(S, D)
    any_spec = pl.BlockSpec(memory_space=pl.ANY)
    out = pl.pallas_call(
        _kernel,
        out_shape=jax.ShapeDtypeStruct((S, D), A_x.dtype),
        in_specs=[any_spec] * 6,
        out_specs=any_spec,
        scratch_shapes=[
            pltpu.VMEM((S, D), _BF16),
            pltpu.VMEM((D, 3 * D), _BF16),
            pltpu.VMEM((D, D), _BF16),
            pltpu.VMEM((D, DFF), _BF16),
            pltpu.VMEM((DFF, D), _BF16),
            pltpu.VMEM((D,), _BF16),
            pltpu.VMEM((S, D), _BF16),
            pltpu.VMEM((2 * NSLAB - 1, S // 2, LANES), _U32),
            pltpu.VMEM((H, LANES // 2, S), _U32),
            pltpu.VMEM((H // 2, 2 * DH, S), _F32),
            pltpu.VMEM((H, 16, S), _U32),
            pltpu.VMEM((H // 2, 2 * DH, S), _F32),
            pltpu.VMEM((NSUB, S, TQ), _F32),
            pltpu.VMEM((NSUB, S, TQ), _F32),
            pltpu.VMEM((NSUB, 8, TQ), _F32),
            pltpu.VMEM((NSUB, 8, TQ), _F32),
            pltpu.VMEM((DH, NV, LANES), _F32),
            pltpu.VMEM((DH, NV, LANES), _F32),
            pltpu.VMEM((DH, 8, S), _F32),
            pltpu.VMEM((DH, 8, S), _F32),
            pltpu.VMEM((D // 2, DFF), _U32),
            pltpu.VMEM((DFF // 2, D), _U32),
            pltpu.VMEM((TF // 2, DFF), _U32),
            pltpu.VMEM((TF // 2, DFF), _U32),
            pltpu.VMEM((S, D), _F32),
            pltpu.VMEM((S, LANES), _F32),
            pltpu.SMEM((1,), jnp.int32),
            pltpu.SemaphoreType.DMA((_NSEM,)),
        ],
        compiler_params=pltpu.CompilerParams(
            vmem_limit_bytes=120 * 1024 * 1024),
    )(x, A_wqkv, A_wo, B_w1, B_w2, gate_w)
    return out.reshape(A_x.shape)
```

```python
import math

import jax
import jax.numpy as jnp
import jax.experimental.pallas as pl
import jax.experimental.pallas.tpu as pltpu

S = 2048
D = 640
H = 32
DH = 20
DFF = 1536
LANES = 128
NSLAB = D // LANES
NFT = DFF // LANES
TQ = 128
NSUB = S // TQ
NV = 272
NG = 2
SAMP = 4
NMR = S - NV
CK = 128
NCK = S // CK
TF = S // H
TP = 512
NP = S // TP
TPQ = 1024
TO = 512
NO = S // TO
TL = 256
QSCALE = (DH ** -0.5) * math.log2(math.e)
SAFE_GAP = 32.0
BOUND_MARGIN = 1.03125

_F32 = jnp.float32
_BF16 = jnp.bfloat16
_U32 = jnp.uint32

_SEM_WK, _SEM_WQ, _SEM_WV, _SEM_WO, _SEM_W1, _SEM_W2, _SEM_GW = range(7)
_SEM_X = 7
_SEM_OUT = _SEM_X + NP
_NSEM = _SEM_OUT + NO + 1


def _pack(x):
    return pltpu.bitcast(x.astype(_BF16), _U32)


def _unpack(x):
    return pltpu.bitcast(x, _BF16)


def _ones_lane(slab):
    if slab == 0:
        return LANES - 2
    return 0 if slab < NSLAB else LANES // 2


def _head_rows(h):
    c0 = h * DH
    j = c0 // LANES
    lo = c0 - j * LANES
    hi = lo + DH
    blocks = {}
    for blk in range(lo // 16, -(-min(hi, LANES) // 16)):
        blocks[blk] = (j * LANES + blk * 16, lo - blk * 16, hi - blk * 16)
    if hi > LANES:
        for blk in range(-(-(hi - LANES) // 16)):
            blocks[blk] = ((j + 1) * LANES + blk * 16, 0,
                           hi - LANES - blk * 16)
    return blocks, _ones_lane(NSLAB + j if hi > LANES else j)


def _kernel(x_hbm, wqkv_hbm, wo_hbm, w1_hbm, w2_hbm, gw_hbm, out_hbm,
            x_v, wqkv_v, wo_v, w1_v, w2_v, out_v,
            kslab, qm_all, qh32, shift, vta, ot, s0, s1, kmax, chk,
            kb0, kb1, qb0, qb1, w1p, w2p, h0, h1, bbuf, gcol, gw_v, zero_s, sems):
    def wcopy(col, slot):
        dst = (0, 2, 1)[col]
        return pltpu.make_async_copy(
            wqkv_hbm.at[:, pl.ds(col * D, D)], wqkv_v.at[:, pl.ds(dst * D, D)],
            sems.at[slot])

    def gate(x, zero):
        z = jnp.tile(zero, (x.shape[0] // 8, x.shape[1] // LANES))
        return pltpu.bitcast(pltpu.bitcast(x, jnp.int32) | z, x.dtype)

    def zero_of(v):
        zmask = jnp.full((8, LANES), zero_s[0], jnp.int32)
        return pltpu.bitcast(v, jnp.int32) & zmask

    def xcopy(t):
        r0 = pl.multiple_of(t * TP, TP)
        return pltpu.make_async_copy(
            x_hbm.at[pl.ds(r0, TP), :], x_v.at[pl.ds(r0, TP), :],
            sems.at[_SEM_X + t])

    def ocopy(t):
        r0 = pl.multiple_of(t * TO, TO)
        return pltpu.make_async_copy(
            out_v.at[pl.ds(r0, TO), :], out_hbm.at[pl.ds(r0, TO), :],
            sems.at[_SEM_OUT + t])

    late = [pltpu.make_async_copy(w1_hbm, w1_v, sems.at[_SEM_W1]),
            pltpu.make_async_copy(w2_hbm, w2_v, sems.at[_SEM_W2]),
            pltpu.make_async_copy(wo_hbm, wo_v, sems.at[_SEM_WO])]
    gwcopy = pltpu.make_async_copy(gw_hbm, gw_v, sems.at[_SEM_GW])

    zero_s[0] = 0
    gwcopy.start()
    wcopy(1, _SEM_WK).start()
    xcopy(0).start()
    xcopy(1).start()

    def zero(h, carry):
        qm_all[h] = jnp.zeros((LANES // 2, S), _U32)
        return carry
    jax.lax.fori_loop(0, H, zero, 0)
    chk[...] = jnp.zeros((NSUB, 8, TQ), _F32)
    kmax[0:H, :] = jnp.zeros((H, LANES), _F32)
    out_v[S - TP:S, :] = jnp.zeros((TP, D), _BF16)

    gwcopy.wait()
    wcopy(1, _SEM_WK).wait()
    xcopy(2).start()
    xcopy(3).start()
    wcopy(0, _SEM_WQ).start()
    wcopy(2, _SEM_WV).start()

    def key_norms(tile):
        col = jax.lax.broadcasted_iota(jnp.int32, (H, D), 1)
        hlo = jax.lax.broadcasted_iota(jnp.int32, (H, D), 0) * DH
        head_sum = jnp.where(jnp.logical_and(col >= hlo, col < hlo + DH),
                             1.0, 0.0).astype(_BF16)
        ksq = out_v[pl.ds(pl.multiple_of(tile * TP, TP), TP), :]
        kn2 = jax.lax.dot_general(head_sum, ksq, (((1,), (1,)), ((), ())),
                                  preferred_element_type=_F32)
        km = kmax[0:H, :]
        for c in range(TP // LANES):
            km = jnp.maximum(km, kn2[:, c * LANES:(c + 1) * LANES])
        return km

    def proj_k(t, carry):
        xcopy(t).wait()
        kmax[0:H, :] = key_norms((t + NP - 1) % NP)
        r0 = pl.multiple_of(t * TP, TP)
        rh = pl.multiple_of(t * (TP // 2), TP // 2)
        xt = x_v[pl.ds(r0, TP), :]
        k = jnp.dot(xt, wqkv_v[:, 2 * D:3 * D], preferred_element_type=_F32)
        lane = jax.lax.broadcasted_iota(jnp.int32, (TP, LANES), 1)
        for j in range(NSLAB):
            kj = k[:, j * LANES:(j + 1) * LANES]
            kslab[j, pl.ds(rh, TP // 2), :] = _pack(
                jnp.where(lane == _ones_lane(j), 1.0, kj))
            if j + 1 < NSLAB:
                kn = k[:, (j + 1) * LANES:(j + 2) * LANES]
                ol = _ones_lane(NSLAB + j)
                kslab[NSLAB + j, pl.ds(rh, TP // 2), :] = _pack(jnp.where(
                    lane > ol, kj, jnp.where(lane == ol, 1.0, kn)))
        out_v[pl.ds(r0, TP), :] = (k * k).astype(_BF16)
        return carry

    jax.lax.fori_loop(0, NP, proj_k, 0)

    wcopy(0, _SEM_WQ).wait()
    wcopy(2, _SEM_WV).wait()
    for cp in late:
        cp.start()

    def proj_qv(t, carry):
        cols = pl.ds(pl.multiple_of(t * TPQ, TPQ), TPQ)
        km = jnp.broadcast_to(
            jnp.max(key_norms(NP - 1), axis=1, keepdims=True), (H, LANES))
        xt = x_v[cols, :]
        tdims = (((0,), (1,)), ((), ()))
        qv_t = jax.lax.dot_general(wqkv_v[:, 0:2 * D], xt, tdims,
                                   preferred_element_type=_F32)
        q_t = qv_t[0:D] * QSCALE
        v_t = qv_t[D:2 * D]
        q_t = q_t.astype(_BF16).astype(_F32)
        qh32[:, :, cols] = q_t.reshape(H // 2, 2 * DH, TPQ)
        row = jax.lax.broadcasted_iota(jnp.int32, (16, TPQ), 0)
        row8 = jax.lax.broadcasted_iota(jnp.int32, (8, TPQ), 0)
        for h in range(H):
            b = 2 * DH * (h // 2)
            sq = [q_t[b + 8 * i:b + 8 * (i + 1)] for i in range(5)]
            sq = [x * x for x in sq]
            if h % 2:
                part = jnp.where(row8 >= 4, sq[2], 0.0) + sq[3] + sq[4]
            else:
                part = sq[0] + sq[1] + jnp.where(row8 < 4, sq[2], 0.0)
            qn2 = jnp.broadcast_to(jnp.sum(part, axis=0, keepdims=True),
                                   (8, TPQ))
            kmh = jnp.broadcast_to(km[h:h + 1], (8, LANES))
            bound = jnp.sqrt(qn2 * jnp.tile(kmh, (1, TPQ // LANES)))
            neg = -((bound * BOUND_MARGIN).astype(_BF16).astype(_F32))
            shift[h, :, cols] = neg
            blocks, srow = _head_rows(h)
            for blk in sorted(set(blocks) | {srow // 16}):
                val = jnp.zeros((16, TPQ), _F32)
                if blk in blocks:
                    src, vlo, vhi = blocks[blk]
                    val = jnp.where(jnp.logical_and(row >= vlo, row < vhi),
                                    q_t[src:src + 16], val)
                if blk == srow // 16:
                    val = jnp.where(row == srow % 16,
                                    jnp.concatenate([neg, neg], axis=0), val)
                qm_all[h, blk * 8:(blk + 1) * 8, cols] = _pack(val)
        ones = jnp.ones((8, TPQ), _F32)
        for p in range(H // 2):
            b = 2 * DH * p
            vta[2 * p, :, cols] = _pack(jnp.concatenate(
                [v_t[b:b + 24], ones], axis=0))
            vta[2 * p + 1, :, cols] = _pack(jnp.concatenate(
                [v_t[b + 16:b + 40], ones], axis=0))
        return carry

    jax.lax.fori_loop(0, S // TPQ, proj_qv, 0)

    def slab_of(h):
        c0 = h * DH
        j = c0 // LANES
        lo = c0 - j * LANES
        return jnp.where(lo + DH > LANES, NSLAB + j, j), lo

    def store_o(pair, odd, cols, acc):
        inv = 1.0 / acc[24:25, :]
        if odd:
            ot[pair, DH:2 * DH, cols] = acc[4:24, :] * inv
        else:
            ot[pair, 0:DH, cols] = acc[0:DH, :] * inv

    def ffn_steps(f1, f2, first):
        facc = [None]

        def step(lhs, w, last):
            def run():
                pr = jnp.dot(lhs(), w(), preferred_element_type=_F32)
                facc[0] = pr if facc[0] is None else facc[0] + pr
                if last is not None:
                    last(facc[0])
                    facc[0] = None
            return run

        g1, g2 = [], []
        if f1 is not None:
            f1r = pl.multiple_of(f1[0] * TF, TF)
            for n in range(NFT):
                lanes = slice(n * LANES, (n + 1) * LANES)

                def fin1(hh, lanes=lanes):
                    f1[1][:, lanes] = _pack(jnp.maximum(hh, 0.0))

                def w1_tile(kt, lanes=lanes):
                    if first:
                        return w1_v[kt * LANES:(kt + 1) * LANES, lanes]
                    return _unpack(w1p[kt * 64:(kt + 1) * 64, lanes])
                g1.append([step(
                    lambda kt=kt: x_v[pl.ds(f1r, TF), kt * LANES:(kt + 1) * LANES],
                    lambda kt=kt, w1_tile=w1_tile: w1_tile(kt),
                    fin1 if kt == NSLAB - 1 else None) for kt in range(NSLAB)])
        if f2 is not None:
            f2r = pl.multiple_of(f2[0] * TF, TF)
            for n in range(NSLAB):
                lanes = slice(n * LANES, (n + 1) * LANES)

                def fin2(bb, lanes=lanes):
                    bbuf[pl.ds(f2r, TF), lanes] = bb
                g2.append([step(
                    lambda kt=kt: _unpack(f2[1][:, kt * LANES:(kt + 1) * LANES]),
                    lambda kt=kt, lanes=lanes: _unpack(
                        w2p[kt * 64:(kt + 1) * 64, lanes]),
                    fin2 if kt == NFT - 1 else None) for kt in range(NFT)])
        steps = []
        while g1 or g2:
            n1 = 3 if len(g2) < 3 else 2
            for grp in g1[:2] + g2[:1] + g1[2:n1]:
                steps += grp
            g1, g2 = g1[n1:], g2[1:]
        return steps

    def stage(a, b, c, steps, subs=range(NSUB), ubase=None, repack=False):
        use_vpu = a is not None and a[2] is not None
        nmr = NMR if use_vpu else S
        nrg = nmr // 8
        npiece = NV // (8 * NG) if use_vpu else 0
        if a is not None:
            ha, s_w, kb_r, qb_r = a
            kidx, _ = slab_of(ha)
        if b is not None:
            hb, b_odd, s_r = b
        prep = []
        if c is not None:
            hc, c_odd, kb_w, qb_w = c
            cidx, clo = slab_of(hc)
            kv = pltpu.roll(
                _unpack(kslab[cidx, NMR // 2:S // 2, :]).astype(_F32),
                (LANES - clo) % LANES, 1)
            w0 = 16 if c_odd else 0
            woff = 4 if c_odd else 0

            def prep_k(d, zero):
                kb_w[d] = jnp.broadcast_to(gate(kv, zero)[:, d:d + 1],
                                           (NV, LANES))

            def prep_q(t, zero):
                lanes = slice(t * LANES, (t + 1) * LANES)
                win = gate(qh32[hc // 2, w0:w0 + 24, lanes], zero)
                for d in range(DH):
                    qb_w[d, :, lanes] = jnp.broadcast_to(
                        win[woff + d:woff + d + 1, :], (8, LANES))

            def prep_w(nj, zero):
                n, j = nj
                a_ = slice(n * LANES, (n + 1) * LANES)
                b_ = slice(j * LANES, (j + 1) * LANES)
                w2p[n * 64:(n + 1) * 64, b_] = gate(
                    pltpu.bitcast(w2_v[a_, b_], _U32), zero)
                w1p[j * 64:(j + 1) * 64, a_] = gate(
                    pltpu.bitcast(w1_v[b_, a_], _U32), zero)

            def prep_g(n, zero):
                tc = 64
                gw = gate(jnp.broadcast_to(
                    gw_v[...].astype(_F32).reshape(1, D), (8, D)), zero)
                xj = x_v[n * tc:(n + 1) * tc, :].astype(_F32)
                z = jnp.sum((xj.reshape(tc // 8, 8, D) * gw[None]).reshape(tc, D),
                            axis=-1, keepdims=True)
                gcol[n * tc:(n + 1) * tc, :] = jnp.broadcast_to(
                    1.0 / (1.0 + jnp.exp(-z)), (tc, LANES))

            lists = [[(prep_k, d) for d in range(DH)],
                     [(prep_q, t) for t in range(S // LANES)]]
            if repack:
                lists.append([(prep_g, n) for n in range(0, S // 64, 2)])
                lists.append([(prep_g, n) for n in range(1, S // 64, 2)])
                for j0 in range(3):
                    lists.append([(prep_w, (n, j)) for n in range(NFT)
                                  for j in range(NSLAB)][j0::3])
            while any(lists):
                for lst in lists:
                    if lst:
                        prep.append(lst.pop(0))
        nprep = len(prep)
        nsub = len(subs)
        pi = 0
        ui = 0
        for un, u in enumerate(subs):
            if ubase is None:
                cols = slice(u * TQ, (u + 1) * TQ)
            else:
                u = ubase + u
                cols = pl.ds(pl.multiple_of(u * TQ, TQ), TQ)
            if a is not None:
                qm = _unpack(qm_all[ha, :, cols])
                macc = [None]

                def piece(w, u=u, cols=cols, macc=macc):
                    gs = range(w * NG, (w + 1) * NG)
                    sv = {g: shift[ha, :, cols] for g in gs}
                    for d in range(DH):
                        qd = qb_r[d, :, cols]
                        for g in gs:
                            sv[g] = kb_r[d, g * 8:(g + 1) * 8, :] * qd + sv[g]
                    for g in gs:
                        s_w[u, NMR + g * 8:NMR + (g + 1) * 8, :] = sv[g]
                        macc[0] = jnp.maximum(macc[0], sv[g])
            acc = None
            wi = 0
            ra = 0
            for ci in range(NCK):
                rows = slice(ci * CK, (ci + 1) * CK)
                if a is not None and ci * CK < nmr:
                    r0, r1 = ci * CK, min((ci + 1) * CK, nmr)
                    s = jnp.dot(_unpack(kslab[kidx, r0 // 2:r1 // 2, :]), qm,
                                preferred_element_type=_F32)
                    s_w[u, r0:r1, :] = s
                    for rg in range((r1 - r0) // 8):
                        v = s[rg * 8:(rg + 1) * 8, :]
                        if ra % SAMP == 0:
                            macc[0] = (v if macc[0] is None
                                       else jnp.maximum(macc[0], v))
                        ra += 1
                        while wi < npiece and wi * nrg < ra * npiece - nrg // 2:
                            piece(wi)
                            wi += 1
                        while (pi < nprep and (pi + 1) * nsub * nrg
                               <= (un * nrg + ra) * (nprep + 2)):
                            fn, arg = prep[pi]
                            fn(arg, zero_of(v))
                            pi += 1
                if b is not None:
                    p = jnp.exp2(s_r[u, rows, :]).astype(_BF16)
                    pv = jnp.dot(_unpack(vta[hb, :, rows]), p,
                                 preferred_element_type=_F32)
                    acc = pv if acc is None else acc + pv
                while (ui < len(steps) and (ui + 1) * nsub * NCK
                       <= (un * NCK + ci + 2) * len(steps)):
                    steps[ui]()
                    ui += 1
            if a is not None:
                while wi < npiece:
                    piece(wi)
                    wi += 1
                safe = jnp.broadcast_to(
                    jnp.max(macc[0], axis=0, keepdims=True),
                    (8, TQ)) >= -SAFE_GAP
                chk[u] = jnp.where(safe, chk[u], 1.0)
            if b is not None:
                store_o(hb // 2, b_odd, cols, acc)
        assert pi == nprep and ui == len(steps)

    late[0].wait()
    late[1].wait()
    stage((0, s0, None, None), None, (1, True, kb1, qb1),
          ffn_steps((0, h0), None, True), repack=True)

    def att(i, carry):
        @pl.when(i % 2 == 0)
        def _():
            hc = jnp.minimum(i + 2, H - 2)
            stage((i + 1, s1, kb1, qb1), (i, False, s0),
                  (hc, False, kb0, qb0), ffn_steps((i + 1, h1), (i, h0), False))

        @pl.when(i % 2 == 1)
        def _():
            stage((i + 1, s0, kb0, qb0), (i, True, s1),
                  (i + 2, True, kb1, qb1), ffn_steps((i + 1, h0), (i, h1), False))
        return carry

    jax.lax.fori_loop(0, H - 1, att, 0)

    unsafe = jnp.max(chk[...].reshape(NSUB * 8, TQ))

    @pl.when(unsafe > 0.0)
    def _():
        def exact(it, carry):
            h = it // NSUB
            u = it % NSUB
            cols = pl.ds(pl.multiple_of(u * TQ, TQ), TQ)
            kidx, _ = slab_of(h)
            srow = jnp.where(
                kidx == 0, _ones_lane(0) // 2,
                jnp.where(kidx < NSLAB, _ones_lane(1) // 2,
                          _ones_lane(NSLAB) // 2))
            prow = jax.lax.broadcasted_iota(jnp.int32, (LANES // 2, TQ), 0)
            qm = _unpack(jnp.where(prow == srow, jnp.uint32(0),
                                   qm_all[h, :, cols]))
            s = jnp.dot(_unpack(kslab[kidx]), qm, preferred_element_type=_F32)
            s = s - jnp.max(s, axis=0, keepdims=True)
            s1[u] = s
            acc = jnp.dot(_unpack(vta[h]), jnp.exp2(s).astype(_BF16),
                          preferred_element_type=_F32)

            @pl.when(h % 2 == 0)
            def _():
                store_o(h // 2, False, cols, acc)

            @pl.when(h % 2 == 1)
            def _():
                store_o(h // 2, True, cols, acc)
            return carry
        jax.lax.fori_loop(0, H * NSUB, exact, 0)

    spt = TO // TQ
    last_b = (H - 1, True, s1)
    stage(None, last_b, None, ffn_steps(None, (H - 1, h1), False),
          subs=range(spt))
    late[2].wait()

    def out_steps(rows, n_rows):
        o_t = ot[:, :, rows].reshape(D, n_rows).astype(_BF16)

        def step(n):
            def run():
                lanes = slice(n * LANES, (n + 1) * LANES)
                g = gcol[rows, :]
                a = jax.lax.dot_general(o_t, wo_v[:, lanes],
                                        (((0,), (0,)), ((), ())),
                                        preferred_element_type=_F32)
                out_v[rows, lanes] = (
                    g * a + (1.0 - g) * bbuf[rows, lanes]).astype(out_v.dtype)
            return run
        return [step(n) for n in range(NSLAB)]

    def outp(t, carry):
        rows = pl.ds(pl.multiple_of(t * TO, TO), TO)
        stage(None, last_b, None, out_steps(rows, TO), subs=range(spt),
              ubase=(t + 1) * spt)
        ocopy(t).start()
        return carry

    jax.lax.fori_loop(0, NO - 1, outp, 0)
    tails = []
    for half, (r0, n_rows) in enumerate(((S - TO, TO - TL), (S - TL, TL))):
        for run in out_steps(slice(r0, r0 + n_rows), n_rows):
            run()
        tails.append(pltpu.make_async_copy(
            out_v.at[pl.ds(r0, n_rows), :], out_hbm.at[pl.ds(r0, n_rows), :],
            sems.at[_SEM_OUT + NO - 1 + half]))
        tails[-1].start()
    for t in range(NO - 1):
        ocopy(t).wait()
    for cp in tails:
        cp.wait()


@jax.jit
def pallas_gated_mix__softmax_full_mha__dense_activation_relu__prompt_kernel(
    A_x: jax.Array,
    A_wqkv: jax.Array,
    A_wo: jax.Array,
    B_x: jax.Array,
    B_w1: jax.Array,
    B_w2: jax.Array,
    gate_w: jax.Array,
):
    del B_x
    x = A_x.reshape(S, D)
    any_spec = pl.BlockSpec(memory_space=pl.ANY)
    out = pl.pallas_call(
        _kernel,
        out_shape=jax.ShapeDtypeStruct((S, D), A_x.dtype),
        in_specs=[any_spec] * 6,
        out_specs=any_spec,
        scratch_shapes=[
            pltpu.VMEM((S, D), _BF16),
            pltpu.VMEM((D, 3 * D), _BF16),
            pltpu.VMEM((D, D), _BF16),
            pltpu.VMEM((D, DFF), _BF16),
            pltpu.VMEM((DFF, D), _BF16),
            pltpu.VMEM((S, D), _BF16),
            pltpu.VMEM((2 * NSLAB - 1, S // 2, LANES), _U32),
            pltpu.VMEM((H, LANES // 2, S), _U32),
            pltpu.VMEM((H // 2, 2 * DH, S), _F32),
            pltpu.VMEM((H, 8, S), _F32),
            pltpu.VMEM((H, 16, S), _U32),
            pltpu.VMEM((H // 2, 2 * DH, S), _F32),
            pltpu.VMEM((NSUB, S, TQ), _F32),
            pltpu.VMEM((NSUB, S, TQ), _F32),
            pltpu.VMEM((4 * H, LANES), _F32),
            pltpu.VMEM((NSUB, 8, TQ), _F32),
            pltpu.VMEM((DH, NV, LANES), _F32),
            pltpu.VMEM((DH, NV, LANES), _F32),
            pltpu.VMEM((DH, 8, S), _F32),
            pltpu.VMEM((DH, 8, S), _F32),
            pltpu.VMEM((D // 2, DFF), _U32),
            pltpu.VMEM((DFF // 2, D), _U32),
            pltpu.VMEM((TF // 2, DFF), _U32),
            pltpu.VMEM((TF // 2, DFF), _U32),
            pltpu.VMEM((S, D), _F32),
            pltpu.VMEM((S, LANES), _F32),
            pltpu.VMEM((D,), _BF16),
            pltpu.SMEM((1,), jnp.int32),
            pltpu.SemaphoreType.DMA((_NSEM,)),
        ],
        compiler_params=pltpu.CompilerParams(
            vmem_limit_bytes=120 * 1024 * 1024),
    )(x, A_wqkv, A_wo, B_w1, B_w2, gate_w)
    return out.reshape(A_x.shape)
```

```python
import math

import jax
import jax.numpy as jnp
import jax.experimental.pallas as pl
import jax.experimental.pallas.tpu as pltpu

S = 2048
D = 640
H = 32
DH = 20
DFF = 1536
LANES = 128
NSLAB = D // LANES
NFT = DFF // LANES
TQ = 128
NSUB = S // TQ
NV = 304
NG = 2
SAMP = 4
NMR = S - NV
CK = 128
NCK = S // CK
TF = S // H
TP = 512
NP = S // TP
TPQ = 1024
TO = 512
NO = S // TO
TL = 256
QSCALE = (DH ** -0.5) * math.log2(math.e)
SAFE_GAP = 32.0
BOUND_MARGIN = 1.03125

_F32 = jnp.float32
_BF16 = jnp.bfloat16
_U32 = jnp.uint32

_SEM_WK, _SEM_WQ, _SEM_WV, _SEM_WO, _SEM_W1, _SEM_W2, _SEM_GW = range(7)
_SEM_X = 7
_SEM_OUT = _SEM_X + NP
_NSEM = _SEM_OUT + NO + 1


def _pack(x):
    return pltpu.bitcast(x.astype(_BF16), _U32)


def _unpack(x):
    return pltpu.bitcast(x, _BF16)


def _ones_lane(slab):
    if slab == 0:
        return LANES - 2
    return 0 if slab < NSLAB else LANES // 2


def _head_rows(h):
    c0 = h * DH
    j = c0 // LANES
    lo = c0 - j * LANES
    hi = lo + DH
    blocks = {}
    for blk in range(lo // 16, -(-min(hi, LANES) // 16)):
        blocks[blk] = (j * LANES + blk * 16, lo - blk * 16, hi - blk * 16)
    if hi > LANES:
        for blk in range(-(-(hi - LANES) // 16)):
            blocks[blk] = ((j + 1) * LANES + blk * 16, 0,
                           hi - LANES - blk * 16)
    return blocks, _ones_lane(NSLAB + j if hi > LANES else j)


def _kernel(x_hbm, wqkv_hbm, wo_hbm, w1_hbm, w2_hbm, gw_hbm, out_hbm,
            x_v, wqkv_v, wo_v, w1_v, w2_v, out_v,
            kslab, qm_all, qh32, shift, vta, ot, s0, s1, kmax, chk,
            kb0, kb1, qb0, qb1, w1p, w2p, h0, h1, bbuf, gcol, xp, gw_v,
            zero_s, sems):
    def wcopy(col, slot):
        dst = (0, 2, 1)[col]
        return pltpu.make_async_copy(
            wqkv_hbm.at[:, pl.ds(col * D, D)], wqkv_v.at[:, pl.ds(dst * D, D)],
            sems.at[slot])

    def gate(x, zero):
        z = jnp.tile(zero, (x.shape[0] // 8, x.shape[1] // LANES))
        return pltpu.bitcast(pltpu.bitcast(x, jnp.int32) | z, x.dtype)

    def zero_of(v):
        zmask = jnp.full((8, LANES), zero_s[0], jnp.int32)
        return pltpu.bitcast(v, jnp.int32) & zmask

    def xcopy(t):
        r0 = pl.multiple_of(t * TP, TP)
        return pltpu.make_async_copy(
            x_hbm.at[pl.ds(r0, TP), :], x_v.at[pl.ds(r0, TP), :],
            sems.at[_SEM_X + t])

    def ocopy(t):
        r0 = pl.multiple_of(t * TO, TO)
        return pltpu.make_async_copy(
            out_v.at[pl.ds(r0, TO), :], out_hbm.at[pl.ds(r0, TO), :],
            sems.at[_SEM_OUT + t])

    late = [pltpu.make_async_copy(w1_hbm, w1_v, sems.at[_SEM_W1]),
            pltpu.make_async_copy(w2_hbm, w2_v, sems.at[_SEM_W2]),
            pltpu.make_async_copy(wo_hbm, wo_v, sems.at[_SEM_WO])]
    gwcopy = pltpu.make_async_copy(gw_hbm, gw_v, sems.at[_SEM_GW])

    zero_s[0] = 0
    gwcopy.start()
    wcopy(1, _SEM_WK).start()
    xcopy(0).start()
    xcopy(1).start()

    def zero(h, carry):
        qm_all[h] = jnp.zeros((LANES // 2, S), _U32)
        return carry
    jax.lax.fori_loop(0, H, zero, 0)
    chk[...] = jnp.zeros((NSUB, 8, TQ), _F32)
    kmax[0:H, :] = jnp.zeros((H, LANES), _F32)
    out_v[S - TP:S, :] = jnp.zeros((TP, D), _BF16)

    gwcopy.wait()
    wcopy(1, _SEM_WK).wait()
    xcopy(2).start()
    xcopy(3).start()
    wcopy(0, _SEM_WQ).start()
    wcopy(2, _SEM_WV).start()

    def key_norms(tile):
        col = jax.lax.broadcasted_iota(jnp.int32, (H, D), 1)
        hlo = jax.lax.broadcasted_iota(jnp.int32, (H, D), 0) * DH
        head_sum = jnp.where(jnp.logical_and(col >= hlo, col < hlo + DH),
                             1.0, 0.0).astype(_BF16)
        ksq = out_v[pl.ds(pl.multiple_of(tile * TP, TP), TP), :]
        kn2 = jax.lax.dot_general(head_sum, ksq, (((1,), (1,)), ((), ())),
                                  preferred_element_type=_F32)
        km = kmax[0:H, :]
        for c in range(TP // LANES):
            km = jnp.maximum(km, kn2[:, c * LANES:(c + 1) * LANES])
        return km

    def proj_k(t, carry):
        xcopy(t).wait()
        kmax[0:H, :] = key_norms((t + NP - 1) % NP)
        r0 = pl.multiple_of(t * TP, TP)
        rh = pl.multiple_of(t * (TP // 2), TP // 2)
        xt = x_v[pl.ds(r0, TP), :]
        k = jnp.dot(xt, wqkv_v[:, 2 * D:3 * D], preferred_element_type=_F32)
        xp[pl.ds(rh, TP // 2), :] = pltpu.bitcast(xt, _U32)
        lane = jax.lax.broadcasted_iota(jnp.int32, (TP, LANES), 1)
        for j in range(NSLAB):
            kj = k[:, j * LANES:(j + 1) * LANES]
            kslab[j, pl.ds(rh, TP // 2), :] = _pack(
                jnp.where(lane == _ones_lane(j), 1.0, kj))
            if j + 1 < NSLAB:
                kn = k[:, (j + 1) * LANES:(j + 2) * LANES]
                ol = _ones_lane(NSLAB + j)
                kslab[NSLAB + j, pl.ds(rh, TP // 2), :] = _pack(jnp.where(
                    lane > ol, kj, jnp.where(lane == ol, 1.0, kn)))
        out_v[pl.ds(r0, TP), :] = (k * k).astype(_BF16)
        return carry

    jax.lax.fori_loop(0, NP, proj_k, 0)

    wcopy(0, _SEM_WQ).wait()
    wcopy(2, _SEM_WV).wait()
    for cp in late:
        cp.start()

    def proj_qv(t, carry):
        cols = pl.ds(pl.multiple_of(t * TPQ, TPQ), TPQ)
        km = jnp.broadcast_to(
            jnp.max(key_norms(NP - 1), axis=1, keepdims=True), (H, LANES))
        xt = x_v[cols, :]
        tdims = (((0,), (1,)), ((), ()))
        qv_t = jax.lax.dot_general(wqkv_v[:, 0:2 * D], xt, tdims,
                                   preferred_element_type=_F32)
        q_t = qv_t[0:D] * QSCALE
        v_t = qv_t[D:2 * D]
        q_t = q_t.astype(_BF16).astype(_F32)
        qh32[:, :, cols] = q_t.reshape(H // 2, 2 * DH, TPQ)
        row = jax.lax.broadcasted_iota(jnp.int32, (16, TPQ), 0)
        row8 = jax.lax.broadcasted_iota(jnp.int32, (8, TPQ), 0)
        for h in range(H):
            b = 2 * DH * (h // 2)
            sq = [q_t[b + 8 * i:b + 8 * (i + 1)] for i in range(5)]
            sq = [x * x for x in sq]
            if h % 2:
                part = jnp.where(row8 >= 4, sq[2], 0.0) + sq[3] + sq[4]
            else:
                part = sq[0] + sq[1] + jnp.where(row8 < 4, sq[2], 0.0)
            qn2 = jnp.broadcast_to(jnp.sum(part, axis=0, keepdims=True),
                                   (8, TPQ))
            kmh = jnp.broadcast_to(km[h:h + 1], (8, LANES))
            bound = jnp.sqrt(qn2 * jnp.tile(kmh, (1, TPQ // LANES)))
            neg = -((bound * BOUND_MARGIN).astype(_BF16).astype(_F32))
            shift[h, :, cols] = neg
            blocks, srow = _head_rows(h)
            for blk in sorted(set(blocks) | {srow // 16}):
                val = jnp.zeros((16, TPQ), _F32)
                if blk in blocks:
                    src, vlo, vhi = blocks[blk]
                    val = jnp.where(jnp.logical_and(row >= vlo, row < vhi),
                                    q_t[src:src + 16], val)
                if blk == srow // 16:
                    val = jnp.where(row == srow % 16,
                                    jnp.concatenate([neg, neg], axis=0), val)
                qm_all[h, blk * 8:(blk + 1) * 8, cols] = _pack(val)
        pad = jnp.ones((8, TPQ), _F32)
        for p in range(H // 2):
            b = 2 * DH * p
            mid = v_t[b + 16:b + 24]
            vta[2 * p, :, cols] = _pack(jnp.concatenate(
                [v_t[b:b + 16], jnp.where(row8 == 4, 1.0, mid), pad], axis=0))
            vta[2 * p + 1, :, cols] = _pack(jnp.concatenate(
                [jnp.where(row8 == 0, 1.0, mid), v_t[b + 24:b + 40], pad],
                axis=0))
        return carry

    jax.lax.fori_loop(0, S // TPQ, proj_qv, 0)

    def slab_of(h):
        c0 = h * DH
        j = c0 // LANES
        lo = c0 - j * LANES
        return jnp.where(lo + DH > LANES, NSLAB + j, j), lo

    def store_o(pair, odd, cols, acc):
        if odd:
            ot[pair, DH:2 * DH, cols] = acc[4:24, :] * (1.0 / acc[0:1, :])
        else:
            ot[pair, 0:DH, cols] = acc[0:DH, :] * (1.0 / acc[DH:DH + 1, :])

    def ffn_steps(f1, f2, first):
        facc = [None]

        def step(lhs, w, last):
            def run():
                pr = jnp.dot(lhs(), w(), preferred_element_type=_F32)
                facc[0] = pr if facc[0] is None else facc[0] + pr
                if last is not None:
                    last(facc[0])
                    facc[0] = None
            return run

        g1, g2 = [], []
        if f1 is not None:
            f1r = pl.multiple_of(f1[0] * (TF // 2), TF // 2)
            for n in range(NFT):
                lanes = slice(n * LANES, (n + 1) * LANES)

                def fin1(hh, lanes=lanes):
                    f1[1][:, lanes] = _pack(jnp.maximum(hh, 0.0))

                def w1_tile(kt, lanes=lanes):
                    if first:
                        return w1_v[kt * LANES:(kt + 1) * LANES, lanes]
                    return _unpack(w1p[kt * 64:(kt + 1) * 64, lanes])
                g1.append([step(
                    lambda kt=kt: _unpack(
                        xp[pl.ds(f1r, TF // 2), kt * LANES:(kt + 1) * LANES]),
                    lambda kt=kt, w1_tile=w1_tile: w1_tile(kt),
                    fin1 if kt == NSLAB - 1 else None) for kt in range(NSLAB)])
        if f2 is not None:
            f2r = pl.multiple_of(f2[0] * TF, TF)
            for n in range(NSLAB):
                lanes = slice(n * LANES, (n + 1) * LANES)

                def fin2(bb, lanes=lanes):
                    bbuf[pl.ds(f2r, TF), lanes] = bb
                g2.append([step(
                    lambda kt=kt: _unpack(f2[1][:, kt * LANES:(kt + 1) * LANES]),
                    lambda kt=kt, lanes=lanes: _unpack(
                        w2p[kt * 64:(kt + 1) * 64, lanes]),
                    fin2 if kt == NFT - 1 else None) for kt in range(NFT)])
        steps = []
        while g1 or g2:
            n1 = 3 if len(g2) < 3 else 2
            for grp in g1[:2] + g2[:1] + g1[2:n1]:
                steps += grp
            g1, g2 = g1[n1:], g2[1:]
        return steps

    def stage(a, b, c, steps, subs=range(NSUB), ubase=None, repack=False):
        use_vpu = a is not None and a[2] is not None
        nmr = NMR if use_vpu else S
        nrg = nmr // 8
        npiece = NV // (8 * NG) if use_vpu else 0
        if a is not None:
            ha, s_w, kb_r, qb_r = a
            kidx, _ = slab_of(ha)
        if b is not None:
            hb, b_odd, s_r = b
        prep = []
        if c is not None:
            hc, c_odd, kb_w, qb_w = c
            cidx, clo = slab_of(hc)
            kv = _unpack(kslab[cidx, NMR // 2:S // 2, :]).astype(_F32)
            w0 = 16 if c_odd else 0
            woff = 4 if c_odd else 0

            def prep_k(d, zero):
                idx = jnp.tile(zero + (clo + d) % LANES, (NV // 8, 1))
                kb_w[d] = jnp.take_along_axis(kv, idx, axis=1)

            def prep_q(t, zero):
                lanes = slice(t * LANES, (t + 1) * LANES)
                win = gate(qh32[hc // 2, w0:w0 + 24, lanes], zero)
                for d in range(DH):
                    qb_w[d, :, lanes] = jnp.broadcast_to(
                        win[woff + d:woff + d + 1, :], (8, LANES))

            def prep_w(nj, zero):
                n, j = nj
                a_ = slice(n * LANES, (n + 1) * LANES)
                b_ = slice(j * LANES, (j + 1) * LANES)
                w2p[n * 64:(n + 1) * 64, b_] = gate(
                    pltpu.bitcast(w2_v[a_, b_], _U32), zero)
                w1p[j * 64:(j + 1) * 64, a_] = gate(
                    pltpu.bitcast(w1_v[b_, a_], _U32), zero)

            def prep_g(n, zero):
                tc = 64
                gw = gate(jnp.broadcast_to(
                    gw_v[...].astype(_F32).reshape(1, D), (8, D)), zero)
                xj = x_v[n * tc:(n + 1) * tc, :].astype(_F32)
                z = jnp.sum((xj.reshape(tc // 8, 8, D) * gw[None]).reshape(tc, D),
                            axis=-1, keepdims=True)
                gcol[n * tc:(n + 1) * tc, :] = jnp.broadcast_to(
                    1.0 / (1.0 + jnp.exp(-z)), (tc, LANES))

            lists = [[(prep_k, d) for d in range(DH)],
                     [(prep_q, t) for t in range(S // LANES)]]
            if repack:
                lists.append([(prep_g, n) for n in range(0, S // 64, 2)])
                lists.append([(prep_g, n) for n in range(1, S // 64, 2)])
                for j0 in range(3):
                    lists.append([(prep_w, (n, j)) for n in range(NFT)
                                  for j in range(NSLAB)][j0::3])
            while any(lists):
                for lst in lists:
                    if lst:
                        prep.append(lst.pop(0))
        nprep = len(prep)
        nsub = len(subs)
        pi = 0
        ui = 0
        for un, u in enumerate(subs):
            if ubase is None:
                cols = slice(u * TQ, (u + 1) * TQ)
            else:
                u = ubase + u
                cols = pl.ds(pl.multiple_of(u * TQ, TQ), TQ)
            if a is not None:
                qm = _unpack(qm_all[ha, :, cols])
                macc = [None]

                if use_vpu:
                    rep = lambda x: jnp.concatenate([x] * NG, axis=0)
                    qd = [rep(qb_r[d, :, cols]) for d in range(DH)]
                    sh = rep(shift[ha, :, cols])

                def piece(w, u=u, macc=macc):
                    keys = slice(w * NG * 8, (w + 1) * NG * 8)
                    sv = sh
                    for d in range(DH):
                        sv = kb_r[d, keys, :] * qd[d] + sv
                    s_w[u, NMR + keys.start:NMR + keys.stop, :] = sv
                    for g in range(NG):
                        macc[0] = jnp.maximum(macc[0], sv[g * 8:(g + 1) * 8])
            acc = None
            wi = 0
            ra = 0
            for ci in range(NCK):
                rows = slice(ci * CK, (ci + 1) * CK)
                if a is not None and ci * CK < nmr:
                    r0, r1 = ci * CK, min((ci + 1) * CK, nmr)
                    s = jnp.dot(_unpack(kslab[kidx, r0 // 2:r1 // 2, :]), qm,
                                preferred_element_type=_F32)
                    s_w[u, r0:r1, :] = s
                    for rg in range((r1 - r0) // 8):
                        if ra % SAMP == 0:
                            v = s[rg * 8:(rg + 1) * 8, :]
                            macc[0] = (v if macc[0] is None
                                       else jnp.maximum(macc[0], v))
                        ra += 1
                        while wi < npiece and wi * nrg < ra * npiece - nrg // 2:
                            piece(wi)
                            wi += 1
                        while (pi < nprep and (pi + 1) * nsub * nrg
                               <= (un * nrg + ra) * (nprep + 4)):
                            fn, arg = prep[pi]
                            fn(arg, zero_of(s[rg * 8:(rg + 1) * 8, :]))
                            pi += 1
                if b is not None:
                    p = jnp.exp2(s_r[u, rows, :]).astype(_BF16)
                    pv = jnp.dot(_unpack(vta[hb, :, rows]), p,
                                 preferred_element_type=_F32)[0:24]
                    acc = pv if acc is None else acc + pv
                while (ui < len(steps) and (ui + 1) * nsub * NCK
                       <= (un * NCK + ci + 4) * len(steps)):
                    steps[ui]()
                    ui += 1
            if a is not None:
                while wi < npiece:
                    piece(wi)
                    wi += 1
                safe = jnp.broadcast_to(
                    jnp.max(macc[0], axis=0, keepdims=True),
                    (8, TQ)) >= -SAFE_GAP
                chk[u] = jnp.where(safe, chk[u], 1.0)
            if b is not None:
                store_o(hb // 2, b_odd, cols, acc)
        assert pi == nprep and ui == len(steps)

    late[0].wait()
    late[1].wait()
    stage((0, s0, None, None), None, (1, True, kb1, qb1),
          ffn_steps((0, h0), None, True), repack=True)

    def att(i, carry):
        @pl.when(i % 2 == 0)
        def _():
            hc = jnp.minimum(i + 2, H - 2)
            stage((i + 1, s1, kb1, qb1), (i, False, s0),
                  (hc, False, kb0, qb0), ffn_steps((i + 1, h1), (i, h0), False))

        @pl.when(i % 2 == 1)
        def _():
            stage((i + 1, s0, kb0, qb0), (i, True, s1),
                  (i + 2, True, kb1, qb1), ffn_steps((i + 1, h0), (i, h1), False))
        return carry

    jax.lax.fori_loop(0, H - 1, att, 0)

    unsafe = jnp.max(chk[...].reshape(NSUB * 8, TQ))

    @pl.when(unsafe > 0.0)
    def _():
        def exact(it, carry):
            h = it // NSUB
            u = it % NSUB
            cols = pl.ds(pl.multiple_of(u * TQ, TQ), TQ)
            kidx, _ = slab_of(h)
            srow = jnp.where(
                kidx == 0, _ones_lane(0) // 2,
                jnp.where(kidx < NSLAB, _ones_lane(1) // 2,
                          _ones_lane(NSLAB) // 2))
            prow = jax.lax.broadcasted_iota(jnp.int32, (LANES // 2, TQ), 0)
            qm = _unpack(jnp.where(prow == srow, jnp.uint32(0),
                                   qm_all[h, :, cols]))
            s = jnp.dot(_unpack(kslab[kidx]), qm, preferred_element_type=_F32)
            s = s - jnp.max(s, axis=0, keepdims=True)
            s1[u] = s
            acc = jnp.dot(_unpack(vta[h]), jnp.exp2(s).astype(_BF16),
                          preferred_element_type=_F32)

            @pl.when(h % 2 == 0)
            def _():
                store_o(h // 2, False, cols, acc)

            @pl.when(h % 2 == 1)
            def _():
                store_o(h // 2, True, cols, acc)
            return carry
        jax.lax.fori_loop(0, H * NSUB, exact, 0)

    spt = TO // TQ
    last_b = (H - 1, True, s1)
    stage(None, last_b, None, ffn_steps(None, (H - 1, h1), False),
          subs=range(spt))
    late[2].wait()

    def out_steps(rows, n_rows):
        o_t = ot[:, :, rows].reshape(D, n_rows).astype(_BF16)

        def step(n):
            def run():
                lanes = slice(n * LANES, (n + 1) * LANES)
                g = gcol[rows, :]
                a = jax.lax.dot_general(o_t, wo_v[:, lanes],
                                        (((0,), (0,)), ((), ())),
                                        preferred_element_type=_F32)
                out_v[rows, lanes] = (
                    g * a + (1.0 - g) * bbuf[rows, lanes]).astype(out_v.dtype)
            return run
        return [step(n) for n in range(NSLAB)]

    def outp(t, carry):
        rows = pl.ds(pl.multiple_of(t * TO, TO), TO)
        stage(None, last_b, None, out_steps(rows, TO), subs=range(spt),
              ubase=(t + 1) * spt)
        ocopy(t).start()
        return carry

    jax.lax.fori_loop(0, NO - 1, outp, 0)
    tails = []
    for half, (r0, n_rows) in enumerate(((S - TO, TO - TL), (S - TL, TL))):
        for run in out_steps(slice(r0, r0 + n_rows), n_rows):
            run()
        tails.append(pltpu.make_async_copy(
            out_v.at[pl.ds(r0, n_rows), :], out_hbm.at[pl.ds(r0, n_rows), :],
            sems.at[_SEM_OUT + NO - 1 + half]))
        tails[-1].start()
    for t in range(NO - 1):
        ocopy(t).wait()
    for cp in tails:
        cp.wait()


@jax.jit
def pallas_gated_mix__softmax_full_mha__dense_activation_relu__prompt_kernel(
    A_x: jax.Array,
    A_wqkv: jax.Array,
    A_wo: jax.Array,
    B_x: jax.Array,
    B_w1: jax.Array,
    B_w2: jax.Array,
    gate_w: jax.Array,
):
    del B_x
    x = A_x.reshape(S, D)
    any_spec = pl.BlockSpec(memory_space=pl.ANY)
    out = pl.pallas_call(
        _kernel,
        out_shape=jax.ShapeDtypeStruct((S, D), A_x.dtype),
        in_specs=[any_spec] * 6,
        out_specs=any_spec,
        scratch_shapes=[
            pltpu.VMEM((S, D), _BF16),
            pltpu.VMEM((D, 3 * D), _BF16),
            pltpu.VMEM((D, D), _BF16),
            pltpu.VMEM((D, DFF), _BF16),
            pltpu.VMEM((DFF, D), _BF16),
            pltpu.VMEM((S, D), _BF16),
            pltpu.VMEM((2 * NSLAB - 1, S // 2, LANES), _U32),
            pltpu.VMEM((H, LANES // 2, S), _U32),
            pltpu.VMEM((H // 2, 2 * DH, S), _F32),
            pltpu.VMEM((H, 8, S), _F32),
            pltpu.VMEM((H, 16, S), _U32),
            pltpu.VMEM((H // 2, 2 * DH, S), _F32),
            pltpu.VMEM((NSUB, S, TQ), _F32),
            pltpu.VMEM((NSUB, S, TQ), _F32),
            pltpu.VMEM((4 * H, LANES), _F32),
            pltpu.VMEM((NSUB, 8, TQ), _F32),
            pltpu.VMEM((DH, NV, LANES), _F32),
            pltpu.VMEM((DH, NV, LANES), _F32),
            pltpu.VMEM((DH, 8, S), _F32),
            pltpu.VMEM((DH, 8, S), _F32),
            pltpu.VMEM((D // 2, DFF), _U32),
            pltpu.VMEM((DFF // 2, D), _U32),
            pltpu.VMEM((TF // 2, DFF), _U32),
            pltpu.VMEM((TF // 2, DFF), _U32),
            pltpu.VMEM((S, D), _F32),
            pltpu.VMEM((S, LANES), _F32),
            pltpu.VMEM((S // 2, D), _U32),
            pltpu.VMEM((D,), _BF16),
            pltpu.SMEM((1,), jnp.int32),
            pltpu.SemaphoreType.DMA((_NSEM,)),
        ],
        compiler_params=pltpu.CompilerParams(
            vmem_limit_bytes=120 * 1024 * 1024),
    )(x, A_wqkv, A_wo, B_w1, B_w2, gate_w)
    return out.reshape(A_x.shape)
```
